```python
import os as _os
_os.environ.setdefault("JAX_PLATFORMS", "cpu")
import jax
import jax.numpy as jnp

def _softmax(x, axis=-1):
    return jax.nn.softmax(x, axis=axis)
def _gelu(x):
    return jax.nn.gelu(x, approximate=True)
def _silu(x):
    return jax.nn.silu(x)
def _sigmoid(x):
    return jax.nn.sigmoid(x)
def _layernorm(x, axis=-1, eps=1e-5):
    m = jnp.mean(x, axis=axis, keepdims=True)
    v = jnp.var(x, axis=axis, keepdims=True)
    return (x - m) / jnp.sqrt(v + eps)
def _scatter_add(tgt, idx, src, axis=0):
    return tgt.at[idx].add(src)
def _segment_sum(src, seg, n):
    return jax.ops.segment_sum(src, seg, n)
class _Rng:
    def __init__(self, key):
        self._k = key
    def _next(self):
        self._k, sub = jax.random.split(self._k)
        return sub
    def normal(self, shape):
        return jax.random.normal(self._next(), shape, dtype=jnp.bfloat16)
    def randint(self, lo, hi, shape):
        return jax.random.randint(self._next(), shape, lo, hi, dtype=jnp.int32)
    def uniform(self, shape, lo=0.0, hi=1.0):
        return jax.random.uniform(self._next(), shape, jnp.bfloat16, lo, hi)
    def permutation(self, n):
        return jax.random.permutation(self._next(), n)


kernel_name = 'standalone__geglu_ffn__prompt'

def setup_inputs():
    _rng = _Rng(jax.random.key(int.from_bytes(__import__("os").urandom(4), "little")))
    _w = (lambda a: (lambda t: t.astype(jnp.bfloat16) if jnp.issubdtype(t.dtype, jnp.floating) else t)(jnp.asarray(a)))
    B, S, D, F = 1, 2048, 576, 4608
    return {
        "x": _w((lambda *s: _rng.normal(s) * 0.05)(B, S, D)),
        "w_gate": _w((lambda *s: _rng.normal(s) * 0.05)(D, F)),
        "w_up": _w((lambda *s: _rng.normal(s) * 0.05)(D, F)),
        "w_down": _w((lambda *s: _rng.normal(s) * 0.05)(F, D)),
    }

def reference(x, w_gate, w_up, w_down):
    return (_gelu(x @ w_gate) * (x @ w_up)) @ w_down
```

```python
import functools

import jax
import jax.numpy as jnp
import jax.experimental.pallas as pl
import jax.experimental.pallas.tpu as pltpu


def _gelu_tanh(x):
    c = 0.7978845608028654
    return 0.5 * x * (1.0 + jnp.tanh(c * (x + 0.044715 * (x * x * x))))


def _kernel(x_ref, wg_ref, wu_ref, wd_ref, o_ref, acc_ref):
    f = pl.program_id(1)

    @pl.when(f == 0)
    def _():
        acc_ref[...] = jnp.zeros_like(acc_ref)

    x = x_ref[...]
    g = jnp.dot(x, wg_ref[...], preferred_element_type=jnp.float32)
    u = jnp.dot(x, wu_ref[...], preferred_element_type=jnp.float32)
    h = (_gelu_tanh(g) * u).astype(jnp.bfloat16)
    acc_ref[...] += jnp.dot(h, wd_ref[...], preferred_element_type=jnp.float32)

    @pl.when(f == pl.num_programs(1) - 1)
    def _():
        o_ref[...] = acc_ref[...].astype(o_ref.dtype)


@jax.jit
def pallas_standalone__geglu_ffn__prompt_kernel(
    x: jax.Array,
    w_gate: jax.Array,
    w_up: jax.Array,
    w_down: jax.Array,
):
    B, S, D = x.shape
    F = w_gate.shape[1]
    M = B * S
    tm, tf = 512, 512
    x2 = x.reshape(M, D)

    out = pl.pallas_call(
        _kernel,
        grid=(M // tm, F // tf),
        in_specs=[
            pl.BlockSpec((tm, D), lambda i, f: (i, 0)),
            pl.BlockSpec((D, tf), lambda i, f: (0, f)),
            pl.BlockSpec((D, tf), lambda i, f: (0, f)),
            pl.BlockSpec((tf, D), lambda i, f: (f, 0)),
        ],
        out_specs=pl.BlockSpec((tm, D), lambda i, f: (i, 0)),
        out_shape=jax.ShapeDtypeStruct((M, D), x.dtype),
        scratch_shapes=[pltpu.VMEM((tm, D), jnp.float32)],
        compiler_params=pltpu.CompilerParams(
            dimension_semantics=("parallel", "arbitrary"),
            vmem_limit_bytes=100 * 1024 * 1024,
        ),
    )(x2, w_gate, w_up, w_down)
    return out.reshape(B, S, D)
```

```python
import functools
import contextlib
import jax
import jax.numpy as jnp
from jax import lax
import jax.experimental.pallas as pl
import jax.experimental.pallas.tpu as pltpu

C0 = 0.7978845608028654
C1 = C0 * 0.044715


def _geglu(g, u):
    z = g * (C0 + C1 * (g * g))
    p = (0.5 * g) * u
    return p + p * jnp.tanh(z)


def build(tf=512, vmem=100, scopes=0, FA=384, NF=3, c0=128, tail=128):
    D, F, M = 576, 4608, 2048
    TM = 512
    MH = 1024
    FB = (F - FA) // NF
    assert FA + NF * FB == F and FB % 128 == 0
    dn_nt = (((1,), (1,)), ((), ()))
    scope = jax.named_scope if scopes else (lambda n: contextlib.nullcontext())
    f32 = jnp.float32

    def chunks(n, tf):
        out, s = [], 0
        while s < n:
            out.append((s, min(tf, n - s)))
            s += tf
        return out

    def kernel(xt_hbm, wg_hbm, wu_hbm, wdt_hbm, o_hbm,
               xt_s, xs, wga, wua, wda, wgb, wub, wdb, acc_s, o_s, sem, osem):
        def cp(src, dst, lo, n, s, dlo=None):
            dlo = lo if dlo is None else dlo
            return pltpu.make_async_copy(src.at[:, pl.ds(lo, n)], dst.at[:, pl.ds(dlo, n)], sem.at[s])

        groups = [
            [cp(xt_hbm, xt_s, 0, TM, 0)],
            [cp(wg_hbm, wga, 0, c0, 1), cp(wu_hbm, wua, 0, c0, 1)],
            [cp(wg_hbm, wga, c0, FA - c0, 2), cp(wu_hbm, wua, c0, FA - c0, 2)],
            [cp(wdt_hbm, wda, 0, FA, 3), cp(xt_hbm, xt_s, TM, TM, 3)],
            [cp(xt_hbm, xt_s, 2 * TM, 2 * TM, 4)],
            [cp(s_, d_.at[0], FA, FB, 5, 0) for s_, d_ in ((wg_hbm, wgb), (wu_hbm, wub), (wdt_hbm, wdb))],
            [cp(s_, d_.at[f], FA + f * FB, FB, 6, 0) for f in range(1, NF)
             for s_, d_ in ((wg_hbm, wgb), (wu_hbm, wub), (wdt_hbm, wdb))],
        ]

        def wait(g):
            for c in groups[g]:
                c.wait()

        for g in groups:
            for c in g:
                c.start()

        def gu(x, wg, wu):
            g = jnp.dot(x, wg, preferred_element_type=f32)
            u = jnp.dot(x, wu, preferred_element_type=f32)
            return _geglu(g, u).astype(jnp.bfloat16)

        def down(wd, h):
            return lax.dot_general(wd, h, dn_nt, preferred_element_type=f32)

        def xpose(t):
            x = xt_s[:, t * TM:(t + 1) * TM].T
            xs[t // 2, (t % 2) * TM:(t % 2 + 1) * TM, :] = x
            return x

        with scope("w0"):
            wait(0)
        x0 = xpose(0)
        with scope("w1"):
            wait(1)
        with scope("s1"):
            h0a = gu(x0, wga[:, 0:c0], wua[:, 0:c0])
        with scope("w2"):
            wait(2)
        with scope("s2"):
            h0b = gu(x0, wga[:, c0:FA], wua[:, c0:FA])
        with scope("w3"):
            wait(3)
        with scope("s3"):
            acc_s[0, :, 0:TM] = down(wda[:, 0:c0], h0a) + down(wda[:, c0:FA], h0b)
            x1 = xpose(1)
            acc_s[0, :, TM:2 * TM] = down(wda[...], gu(x1, wga[...], wua[...]))
        with scope("w4"):
            wait(4)
        with scope("s4"):
            for t in (2, 3):
                xt_ = xpose(t)
                acc_s[1, :, (t - 2) * TM:(t - 1) * TM] = down(wda[...], gu(xt_, wga[...], wua[...]))
        with scope("w5"):
            wait(5)

        def ocp(m, lo, n, s):
            return pltpu.make_async_copy(
                o_s.at[m, :, pl.ds(lo, n)],
                o_hbm.at[:, pl.ds(pl.multiple_of(m * MH + lo, 128), n)], osem.at[s])

        pieces = [(0, TM), (TM, TM - tail), (MH - tail, tail)] if tail < TM else [(0, TM), (TM, TM)]

        def body(j, carry):
            f = j // 2
            m = j % 2

            @pl.when(j == 1)
            def _():
                wait(6)

            last = f == NF - 1
            with scope("body"):
                for t in range(MH // TM):
                    x = xs[m, t * TM:(t + 1) * TM, :]
                    acc = acc_s[m, :, t * TM:(t + 1) * TM]
                    cks = chunks(FB, tf)
                    for ci, (s, n) in enumerate(cks):
                        h = gu(x, wgb[f, :, s:s + n], wub[f, :, s:s + n])
                        if ci < len(cks) - 1:
                            acc = acc + down(wdb[f, :, s:s + n], h)
                        else:
                            for (lo, nn) in pieces:
                                if not (t * TM <= lo < (t + 1) * TM):
                                    continue
                                l0 = lo - t * TM
                                a = acc[:, l0:l0 + nn] + down(wdb[f, :, s:s + n], h[l0:l0 + nn, :])
                                acc_s[m, :, lo:lo + nn] = a
                                o_s[m, :, lo:lo + nn] = a.astype(o_s.dtype)

                                @pl.when(last)
                                def _():
                                    ocp(m, lo, nn, 0).start()
            return carry

        lax.fori_loop(0, 2 * NF, body, 0)
        with scope("owait"):
            for m in range(2):
                for (lo, nn) in pieces:
                    ocp(m, lo, nn, 0).wait()

    def fn(x, w_gate, w_up, w_down):
        B, S, _ = x.shape
        xt = x.reshape(M, D).T
        wdt = w_down.T
        bf = jnp.bfloat16
        out = pl.pallas_call(
            kernel,
            in_specs=[pl.BlockSpec(memory_space=pl.ANY)] * 4,
            out_specs=pl.BlockSpec(memory_space=pl.ANY),
            out_shape=jax.ShapeDtypeStruct((D, M), x.dtype),
            scratch_shapes=[pltpu.VMEM((D, M), bf), pltpu.VMEM((2, MH, D), bf),
                            pltpu.VMEM((D, FA), bf), pltpu.VMEM((D, FA), bf), pltpu.VMEM((D, FA), bf),
                            pltpu.VMEM((NF, D, FB), bf), pltpu.VMEM((NF, D, FB), bf), pltpu.VMEM((NF, D, FB), bf),
                            pltpu.VMEM((2, D, MH), f32), pltpu.VMEM((2, D, MH), bf),
                            pltpu.SemaphoreType.DMA((7,)), pltpu.SemaphoreType.DMA((1,))],
            compiler_params=pltpu.CompilerParams(
                vmem_limit_bytes=vmem * 1024 * 1024,
            ),
        )(xt, w_gate, w_up, wdt)
        return out.T.reshape(B, S, D)
    return fn


_impl = build()


@jax.jit
def pallas_standalone__geglu_ffn__prompt_kernel(
    x: jax.Array,
    w_gate: jax.Array,
    w_up: jax.Array,
    w_down: jax.Array,
):
    return _impl(x, w_gate, w_up, w_down)
```

```python
import functools
import contextlib
import jax
import jax.numpy as jnp
from jax import lax
import jax.experimental.pallas as pl
import jax.experimental.pallas.tpu as pltpu

C0 = 0.7978845608028654
C1 = C0 * 0.044715


def _geglu(g, u):
    z = g * (C0 + C1 * (g * g))
    p = (0.5 * g) * u
    return p + p * jnp.tanh(z)


def build(tf=512, vmem=100, scopes=0, ndb=1, nobc=0, nosc=0, r2a='256', r2b='256', r3a='512', r3b='512', r4='512',
          lastsplit=0, r1="256"):
    D, F, M = 576, 4608, 2048
    TM = 512
    FA, NF, MH = 384, 3, 1024
    NM = M // MH
    TPH = MH // TM
    FB = (F - FA) // NF
    dn_nt = (((1,), (1,)), ((), ()))
    scope = jax.named_scope if scopes else (lambda n: contextlib.nullcontext())
    f32 = jnp.float32
    psz = [TM] * (TPH - 1) + [128] * (TM // 128)
    pieces = [(sum(psz[:i]), psz[i]) for i in range(len(psz))]
    NP = len(pieces)
    NIT = NM * NF
    rows = lambda s: [int(v) for v in str(s).split(',')]

    def chunks(n, tf):
        out, s = [], 0
        if n % tf:
            out.append((0, n % tf))
            s = n % tf
        while s < n:
            out.append((s, tf))
            s += tf
        return out

    def kernel(xt_hbm, wg_hbm, wu_hbm, wdt_hbm, o_hbm,
               xt_s, xs, wga, wua, wda, wgb, wub, wdb, acc_s, *rest):
        o_p = rest[:NP]
        sem, osem = rest[NP:]

        def cp(src, dst, lo, n, s, dlo=None):
            dlo = lo if dlo is None else dlo
            return pltpu.make_async_copy(src.at[:, pl.ds(lo, n)], dst.at[:, pl.ds(dlo, n)], sem.at[s])

        def wb(f, s):
            return [cp(s_, d_.at[f], FA + f * FB, FB, s, 0)
                    for s_, d_ in ((wg_hbm, wgb), (wu_hbm, wub), (wdt_hbm, wdb))]

        def gua(c, s):
            return [cp(wg_hbm, wga, c * 128, 128, s), cp(wu_hbm, wua, c * 128, 128, s)]

        groups = [
            [cp(xt_hbm, xt_s, 0, 256, 0)],
            gua(0, 1),
            gua(1, 2) + [cp(xt_hbm, xt_s, 256, 256, 2)],
            gua(2, 3) + [cp(xt_hbm, xt_s, TM, TM, 3)],
            [cp(wdt_hbm, wda, 0, FA, 4), cp(xt_hbm, xt_s, 2 * TM, 2 * TM, 4)],
            wb(0, 5),
            [c for f in range(1, NF) for c in wb(f, 6)],
        ]

        def wait(g):
            for c in groups[g]:
                c.wait()

        for g in groups:
            for c in g:
                c.start()

        def gu(x, wg, wu):
            g = jnp.dot(x, wg, preferred_element_type=f32)
            u = jnp.dot(x, wu, preferred_element_type=f32)
            return _geglu(g, u).astype(jnp.bfloat16)

        def gu_rows(x, lo, n, rws):
            hs, r0 = [], 0
            wg, wu = wga[:, lo:lo + n], wua[:, lo:lo + n]
            while r0 < x.shape[0]:
                for r in rws:
                    hs.append(gu(x[r0:r0 + r], wg, wu))
                    r0 += r
            return jnp.concatenate(hs, axis=0) if len(hs) > 1 else hs[0]

        def down(wd, h):
            return lax.dot_general(wd, h, dn_nt, preferred_element_type=f32)

        def xpose(lo, n):
            x = xt_s[:, lo:lo + n].T
            xs[lo // MH, lo % MH:lo % MH + n, :] = x
            return x

        def acc_store(t, v):
            acc_s[t // TPH, :, (t % TPH) * TM:(t % TPH + 1) * TM] = v

        def phase_a():
            with scope("w0"):
                wait(0)
            xa = xpose(0, 256)
            with scope("w1"):
                wait(1)
            with scope("s1"):
                ha0 = gu_rows(xa, 0, 128, rows(r1))
            with scope("w2"):
                wait(2)
            with scope("s2"):
                xb = xpose(256, 256)
                ha1 = gu_rows(xa, 128, 128, rows(r2a))
                hb01 = gu_rows(xb, 0, 256, rows(r2b))
            with scope("w3"):
                wait(3)
            with scope("s3"):
                x1 = xpose(TM, TM)
                x0 = jnp.concatenate([xa, xb], axis=0)
                h02 = gu_rows(x0, 256, 128, rows(r3a))
                h1 = gu_rows(x1, 0, FA, rows(r3b))
            with scope("w4"):
                wait(4)
            with scope("s4"):
                h0 = jnp.concatenate(
                    [jnp.concatenate([jnp.concatenate([ha0, ha1], axis=1), hb01], axis=0), h02], axis=1)
                x2 = xpose(2 * TM, TM)
                acc_store(0, down(wda[...], h0))
                x3 = xpose(3 * TM, TM)
                acc_store(1, down(wda[...], h1))
                h2 = gu_rows(x2, 0, FA, rows(r4))
                h3 = gu_rows(x3, 0, FA, rows(r4))
                acc_store(2, down(wda[...], h2))
                acc_store(3, down(wda[...], h3))
            with scope("w5"):
                wait(5)

        def ocp(mm, p):
            lo, n = pieces[p]
            db = p >= NP - ndb
            src = o_p[p].at[mm] if db else o_p[p]
            return pltpu.make_async_copy(src, o_hbm.at[:, pl.ds(mm * MH + lo, n)],
                                         osem.at[1 if (db or mm == NM - 1) else 0])

        def body(j):
            f = lax.shift_right_logical(j, 1)
            m = lax.bitwise_and(j, 1)

            @pl.when(j == 1)
            def _():
                wait(6)

            @pl.when(j > NIT - NM)
            def _():
                for p in range(NP - ndb):
                    ocp(0, p).wait()

            with scope("body"):
                for t in range(TPH):
                    x = xs[m, t * TM:(t + 1) * TM, :]
                    acc = acc_s[m, :, t * TM:(t + 1) * TM]
                    cks = chunks(FB, tf)
                    for ci, (s, n) in enumerate(cks):
                        h = gu(x, wgb[f, :, s:s + n], wub[f, :, s:s + n])
                        acc = acc + down(wdb[f, :, s:s + n], h)
                    for p, (lo, nn) in enumerate(pieces):
                        if not (t * TM <= lo < (t + 1) * TM):
                            continue
                        l0 = lo - t * TM
                        a = acc[:, l0:l0 + nn]
                        acc_s[m, :, lo:lo + nn] = a
                        if p >= NP - ndb:
                            o_p[p][m] = a.astype(jnp.bfloat16)
                        else:
                            o_p[p][...] = a.astype(jnp.bfloat16)
                        for mm in reversed(range(NM)):
                            @pl.when(j == NIT - NM + mm)
                            def _():
                                ocp(mm, p).start()

        def outer(it, carry):
            lax.cond(it == 0, phase_a, lambda: body(it - 1))
            return carry
        lax.fori_loop(0, NIT + 1, outer, 0)

        with scope("owait"):
            for mm in range(NM - 1):
                for p in range(NP - ndb, NP):
                    ocp(mm, p).wait()
            for p in range(NP):
                ocp(NM - 1, p).wait()

    def fn(x, w_gate, w_up, w_down):
        B, S, _ = x.shape
        xt = x.reshape(M, D).T
        wdt = w_down.T
        bf = jnp.bfloat16
        out = pl.pallas_call(
            kernel,
            in_specs=[pl.BlockSpec(memory_space=pl.ANY)] * 4,
            out_specs=pl.BlockSpec(memory_space=pl.ANY),
            out_shape=jax.ShapeDtypeStruct((D, M), x.dtype),
            scratch_shapes=[pltpu.VMEM((D, M), bf), pltpu.VMEM((NM, MH, D), bf),
                            pltpu.VMEM((D, FA), bf), pltpu.VMEM((D, FA), bf), pltpu.VMEM((D, FA), bf),
                            pltpu.VMEM((NF, D, FB), bf), pltpu.VMEM((NF, D, FB), bf), pltpu.VMEM((NF, D, FB), bf),
                            pltpu.VMEM((NM, D, MH), f32)]
                           + [pltpu.VMEM((NM, D, n) if p >= NP - ndb else (D, n), bf)
                              for p, (_, n) in enumerate(pieces)]
                           + [pltpu.SemaphoreType.DMA((7,)), pltpu.SemaphoreType.DMA((2,))],
            compiler_params=pltpu.CompilerParams(
                vmem_limit_bytes=vmem * 1024 * 1024,
                disable_bounds_checks=bool(nobc),
                disable_semaphore_checks=bool(nosc),
            ),
        )(xt, w_gate, w_up, wdt)
        return out.T.reshape(B, S, D)
    return fn


_impl = build(r1='128', r2a='128')


@jax.jit
def pallas_standalone__geglu_ffn__prompt_kernel(
    x: jax.Array,
    w_gate: jax.Array,
    w_up: jax.Array,
    w_down: jax.Array,
):
    return _impl(x, w_gate, w_up, w_down)
```

```python
import contextlib
import jax
import jax.numpy as jnp
from jax import lax
import jax.experimental.pallas as pl
import jax.experimental.pallas.tpu as pltpu

C0 = 0.7978845608028654
C1 = C0 * 0.044715


def _geglu(g, u):
    z = g * (C0 + C1 * (g * g))
    p = (0.5 * g) * u
    return p + p * jnp.tanh(z)


def build(vmem=110, scopes=0, r=128, R=32, lead=8, wt=58, wg_=52, wu_=36, wd_=52, wd4=52, front=0.985,
          lk=4, omode=0, a_front=0.9):
    D, F, M = 576, 4608, 2048
    KM, KT = 512, 64
    TM = 512
    FA, NF, MH = 384, 3, 1024
    NM = M // MH
    TPH = MH // TM
    FB = (F - FA) // NF
    NTA = FA // 128
    NTB = FB // 128
    NQ = TPH * NTB * 2
    ndb = 1
    RM = TM - r
    dn_nt = (((1,), (1,)), ((), ()))
    scope = jax.named_scope if scopes else (lambda n: contextlib.nullcontext())
    f32 = jnp.float32
    bf = jnp.bfloat16
    u32 = jnp.uint32
    psz = [TM] * (TPH - 1) + [128] * (TM // 128)
    pieces = [(sum(psz[:i]), psz[i]) for i in range(len(psz))]
    NP = len(pieces)
    NIT = NM * NF
    CH = [(0, 3), (3, 4), (7, 4)]
    assert r % R == 0 and RM % 32 == 0 and R % 32 == 0

    def kernel(xt_hbm, wg_hbm, wu_hbm, wdt_hbm, o_hbm,
               xt_s, xs, wga, wua, wda, wgb, wub, wdb, acc_s, w32, xb_s, t_s, g_s, h_s, wdp, ha_s, *rest):
        o_p = rest[:NP]
        sem, osem = rest[NP:]

        def cp(src, dst, lo, n, s):
            return pltpu.make_async_copy(src.at[:, pl.ds(lo, n)], dst.at[:, pl.ds(lo, n)], sem.at[s])

        def cpr(src, dst, f, r0, nr, s):
            return pltpu.make_async_copy(src.at[pl.ds(r0, nr), pl.ds(FA + f * FB, FB)],
                                         dst.at[f, pl.ds(r0, nr), :], sem.at[s])

        def wb(f, s):
            return [cpr(wg_hbm, wgb, f, 0, KM, s), cpr(wu_hbm, wub, f, 0, KM, s), cpr(wdt_hbm, wdb, f, 0, D, s)]

        def gua(c, s):
            return [cp(wg_hbm, wga, c * 128, 128, s), cp(wu_hbm, wua, c * 128, 128, s)]

        groups = [
            [cp(xt_hbm, xt_s, 0, 256, 0)],
            gua(0, 1),
            gua(1, 2) + [cp(xt_hbm, xt_s, 256, 256, 2)],
            gua(2, 3) + [cp(xt_hbm, xt_s, TM, TM, 3)],
            [cp(wdt_hbm, wda, 0, FA, 4), cp(xt_hbm, xt_s, 2 * TM, 2 * TM, 4)]
            + [cpr(s_, d_, f, KM, KT, 4) for f in range(NF) for s_, d_ in ((wg_hbm, wgb), (wu_hbm, wub))],
            wb(0, 5),
            [c for f in range(1, NF) for c in wb(f, 6)],
        ]

        def wait(g):
            for c in groups[g]:
                c.wait()

        for g in groups:
            for c in g:
                c.start()

        def mm(a, b):
            return jnp.dot(a, b, preferred_element_type=f32)

        def down(wd, h):
            return lax.dot_general(wd, h, dn_nt, preferred_element_type=f32)

        def xpose(lo, n):
            x = xt_s[:, lo:lo + n].T
            t, r0 = lo // TM, (lo % TM) // 2
            for kt in range(4):
                xs[t, kt, r0:r0 + n // 2, :] = pltpu.bitcast(x[:, kt * 128:(kt + 1) * 128], u32)
            xs[t, 4, r0:r0 + n // 2, :] = jnp.concatenate(
                [pltpu.bitcast(x[:, KM:D], u32), jnp.zeros((n // 2, 128 - KT), u32)], axis=1)
            return x

        def xmain(tt):
            return jnp.concatenate([pltpu.bitcast(xs[tt, kt], bf) for kt in range(4)], axis=1)

        def xtail(tt, a, n):
            return pltpu.bitcast(xs[tt, 4, a // 2:(a + n) // 2, 0:KT], bf)

        class Ties:
            def __init__(self, it, jobs, total_w, front, lumps=(), n_ties=None):
                self.mask = lax.broadcasted_iota(jnp.int32, (R, 128), 1) < (it - 1000)
                self.jobs, self.W, self.front = jobs, total_w, front
                self.total = len(jobs) * (r // R) * KT
                self.w = 0.0
                self.done = self.i = self.r0 = self.k = 0
                self.acc = None
                self.lumps = list(lumps)
                self.w0 = 0.0

            def __call__(self, piece, w):
                self.w += w
                if self.lumps and self.w >= self.lumps[0][0] * self.W:
                    self.lumps.pop(0)[1](piece)
                frac = (self.w - self.w0) / (self.W * self.front - self.w0)
                target = max(0, min(self.total, int(self.total * frac)))
                kk = min(target - self.done, KT - self.k)
                if kk <= 0:
                    return piece
                tile, f, which, n, slot = self.jobs[self.i]
                cs = pl.ds(n * 128, 128)
                acc = self.acc
                for k in range(self.k, self.k + kk):
                    p = xb_s[tile, k, pl.ds(self.r0, R), :] * w32[which, f, pl.ds(k, 1), cs]
                    acc = p if acc is None else acc + p
                self.done += kk
                self.k += kk
                self.acc = acc
                if self.k == KT:
                    t_s[slot, pl.ds(RM + self.r0, R), :] = jnp.where(self.mask, piece, acc)
                    self.k, self.acc = 0, None
                    self.r0 += R
                    if self.r0 == r:
                        self.r0 = 0
                        self.i += 1
                    return piece
                return jnp.where(self.mask, acc, piece)

            def all(self, res, w_per_beat):
                outs = [self(res[a:a + R], w_per_beat * (R // 16)) for a in range(0, res.shape[0] - R + 1, R)]
                rem = res.shape[0] % R
                if rem:
                    self.w += w_per_beat * (rem // 16)
                    outs.append(res[res.shape[0] - rem:])
                return jnp.concatenate(outs, axis=0) if len(outs) > 1 else outs[0]

            def finish(self):
                assert self.done == self.total and not self.lumps, (self.done, self.total, len(self.lumps))

        def ntile(tie, tt, q, wg, wu, rm, h_dst, par, ready=None):
            H = rm // 2
            res = [mm(xtail(tt, 0, H), wg(KM, D)), mm(xtail(tt, H, H), wg(KM, D)),
                   mm(xtail(tt, 0, H), wu(KM, D)), mm(xtail(tt, H, H), wu(KM, D))]
            for a in range(0, H, R):
                n_ = min(R, H - a)
                for i in range(4):
                    v = res[i][a:a + n_]
                    if n_ == R:
                        v = tie(v, wt * (R // 16) / 4)
                    else:
                        tie.w += wt * (n_ // 16) / 4
                    t_s[q + i // 2, pl.ds((i % 2) * H + a, n_), :] = v
            gmain = mm(xmain(tt), wg(0, KM))
            g_s[par, 0:rm] = tie.all(gmain[0:rm] + t_s[q, 0:rm], wg_)
            if rm < TM:
                assert ready(q)
                g_s[par, rm:TM] = tie.all(gmain[rm:TM] + t_s[q, rm:TM], wg_)
            umain = mm(xmain(tt), wu(0, KM))
            u = tie.all(umain[0:rm] + t_s[q + 1, 0:rm], wu_)
            if rm < TM:
                assert ready(q + 1)
                u1 = tie.all(umain[rm:TM] + t_s[q + 1, rm:TM], wu_)
                u = jnp.concatenate([u, u1], axis=0)
            h_dst[...] = pltpu.bitcast(_geglu(g_s[par], u).astype(bf), u32)

        def down4(tie, wd, h_u32, acc_ref, first):
            p_ = down(wd, pltpu.bitcast(h_u32, bf))
            for r0 in range(0, D, R):
                rr_ = min(R, D - r0)
                for a in range(TM // 128):
                    v = p_[r0:r0 + rr_, a * 128:(a + 1) * 128]
                    if not first:
                        v = acc_ref[r0:r0 + rr_, a * 128:(a + 1) * 128] + v
                    if rr_ == R:
                        v = tie(v, wd4 * (R // 16) / 4)
                    else:
                        tie.w += wd4 * (rr_ // 16) / 4
                    acc_ref[r0:r0 + rr_, a * 128:(a + 1) * 128] = v

        w_nt = lambda rm: wt * (rm // 32) + (wg_ + wu_) * (TM // 16)
        w_d4 = wd4 * (D // 16)
        w_dn = wd_ * (D // 16)

        def xb_lump(tie, t, g0, k0):
            def emit(piece):
                src = xs[t, 4, pl.ds(RM // 2 + g0, R), :]
                src = jnp.where(tie.mask, pltpu.bitcast(piece, u32), src)
                for k in range(k0, k0 + lk):
                    b = jnp.broadcast_to(src[:, k:k + 1], (R, 128))
                    xb_s[t, k, pl.ds(2 * g0, 2 * R), :] = pltpu.bitcast(b, bf).astype(f32)
            return emit

        def xb_lumps(tie, t):
            return [xb_lump(tie, t, g0, k0) for k0 in range(0, KT, lk) for g0 in range(0, r // 2, R)]

        def w32_lump(tie, f, which, n):
            def emit(piece):
                cs = pl.ds(n * 128, 128)
                src = pltpu.bitcast((wgb, wub)[which][f, KM:D, cs], u32)
                src = jnp.where(tie.mask[0:KT // 2], pltpu.bitcast(piece[0:KT // 2], u32), src)
                w32[which, f, :, cs] = pltpu.bitcast(src, bf).astype(f32)
            return emit

        def spread(ls, a, b):
            return [(a + (b - a) * i / len(ls), l) for i, l in enumerate(ls)]

        def tail_job(q, m, f):
            t, n, which = q // (2 * NTB), (q % (2 * NTB)) // 2, q % 2
            return (m * TPH + t, f, which, n, q)

        def phase_a(it):
            def gu_v(x, lo, n, rr, t, r0):
                wg, wu = wga[:, lo:lo + n], wua[:, lo:lo + n]
                for a in range(0, x.shape[0], rr):
                    h = _geglu(mm(x[a:a + rr], wg), mm(x[a:a + rr], wu)).astype(bf)
                    for c in range(n // 128):
                        ha_s[t, lo // 128 + c, (r0 + a) // 2:(r0 + a + rr) // 2, :] = pltpu.bitcast(
                            h[:, c * 128:(c + 1) * 128], u32)

            def nt_a(tie, tt, n, cnt):
                cs = pl.ds(n * 128, 128)
                ntile(tie, tt, NQ - 4 + 2 * (cnt % 2), lambda a, b: wga[a:b, cs], lambda a, b: wua[a:b, cs],
                      TM, ha_s.at[tt, n], cnt % 2)

            def dn_a(tie, tt):
                accv = acc_s.at[tt // TPH, :, (tt % TPH) * TM:(tt % TPH + 1) * TM]
                for n in range(NTA):
                    down4(tie, wda[:, n * 128:(n + 1) * 128], ha_s[tt, n], accv, n == 0)

            with scope("w0"):
                wait(0)
            xa = xpose(0, 256)
            with scope("w1"):
                wait(1)
            with scope("s1"):
                gu_v(xa, 0, 128, 128, 0, 0)
            with scope("w2"):
                wait(2)
            with scope("s2"):
                xb = xpose(256, 256)
                gu_v(xa, 128, 128, 128, 0, 0)
                gu_v(xb, 0, 256, 256, 0, 256)
            with scope("w3"):
                wait(3)
            with scope("s3"):
                tie = Ties(it, [], 4 * w_nt(TM), 1.0)
                if r:
                    tie.lumps = spread(xb_lumps(tie, 0), 0.2, 0.95)
                xpose(TM, TM)
                nt_a(tie, 0, 2, 0)
                for n in range(NTA):
                    nt_a(tie, 1, n, n + 1)
                tie.finish()
            with scope("w4"):
                wait(4)
            with scope("s4"):
                jobs = [tail_job(q, 0, 0) for q in range(lead)] if r else []
                tie = Ties(it, jobs, 2 * NTA * w_nt(TM) + 4 * NTA * w_d4, a_front)
                if r:
                    l0 = [w32_lump(tie, 0, which, n) for n in range(NTB) for which in range(2)]
                    l1 = [w32_lump(tie, f, which, n) for f in range(1, NF) for n in range(NTB) for which in range(2)]
                    lx = xb_lumps(tie, 1) + xb_lumps(tie, 2) + xb_lumps(tie, 3)
                    tie.lumps = sorted(spread(l0, 0.0, 0.06) + spread(l1, 0.06, 0.2) + spread(lx, 0.15, 0.95),
                                       key=lambda e: e[0])
                    tie.w0 = 0.1 * tie.W
                xpose(2 * TM, TM)
                dn_a(tie, 0)
                xpose(3 * TM, TM)
                dn_a(tie, 1)
                for tt in (2, 3):
                    for n in range(NTA):
                        nt_a(tie, tt, n, tt * NTA + n)
                dn_a(tie, 2)
                dn_a(tie, 3)
                tie.finish()
            with scope("w5"):
                wait(5)

        def ocp(mm_, p):
            lo, n = pieces[p]
            db = p >= NP - ndb
            src = o_p[p].at[mm_] if db else o_p[p]
            return pltpu.make_async_copy(src, o_hbm.at[:, pl.ds(mm_ * MH + lo, n)],
                                         osem.at[1 if (db or mm_ == NM - 1) else 0])

        def body(j):
            f = lax.shift_right_logical(j, 1)
            m = lax.bitwise_and(j, 1)
            jn = jnp.minimum(j + 1, NIT - 1)
            fn_ = lax.shift_right_logical(jn, 1)
            mn = lax.bitwise_and(jn, 1)

            @pl.when(j == 1)
            def _():
                wait(6)

            @pl.when(j > NIT - NM)
            def _():
                for p in range(NP - ndb):
                    ocp(0, p).wait()

            jobs = ([tail_job(q, m, f) for q in range(lead, NQ)] + [tail_job(q, mn, fn_) for q in range(lead)]) \
                if r else []
            W = TPH * (NTB * w_nt(RM) + sum(nn * (w_dn if nn == 4 else w_d4) for _, nn in CH))
            tie = Ties(j, jobs, W, front)
            ready = lambda q: q < lead + tie.i

            with scope("body"):
                for t in range(TPH):
                    tt = m * TPH + t
                    accv = acc_s.at[m, :, t * TM:(t + 1) * TM]
                    for ci, (n0, nn) in enumerate(CH):
                        for n in range(n0, n0 + nn):
                            cs = pl.ds(n * 128, 128)
                            ntile(tie, tt, (t * NTB + n) * 2, lambda a, b: wgb[f, a:b, cs],
                                  lambda a, b: wub[f, a:b, cs], RM, h_s.at[n], n % 2, ready)
                        if nn != 4:
                            for n in range(n0, n0 + nn):
                                if t == 0:
                                    wd = wdb[f, :, n * 128:(n + 1) * 128]
                                    wdp[n] = pltpu.bitcast(wd, u32)
                                else:
                                    wd = pltpu.bitcast(wdp[n], bf)
                                down4(tie, wd, h_s[n], accv, False)
                            continue
                        for a in range(TM // 128):
                            if t == 0 and a == 0:
                                wd = wdb[f, :, n0 * 128:(n0 + nn) * 128]
                                for n in range(nn):
                                    wdp[n0 + n] = pltpu.bitcast(wd[:, n * 128:(n + 1) * 128], u32)
                            else:
                                wd = jnp.concatenate([pltpu.bitcast(wdp[n], bf) for n in range(n0, n0 + nn)], axis=1)
                            h = jnp.concatenate([pltpu.bitcast(h_s[n, a * 64:(a + 1) * 64, :], bf)
                                                 for n in range(n0, n0 + nn)], axis=1)
                            lo = t * TM + a * 128
                            acc = tie.all(accv[:, a * 128:(a + 1) * 128] + down(wd, h), wd_)
                            accv[:, a * 128:(a + 1) * 128] = acc
                            if ci == len(CH) - 1:
                                p = [i for i, (plo, pn) in enumerate(pieces) if plo <= lo < plo + pn][0]
                                plo, pn = pieces[p]
                                if p >= NP - ndb:
                                    o_p[p][m, :, lo - plo:lo - plo + 128] = acc.astype(bf)
                                else:
                                    o_p[p][:, lo - plo:lo - plo + 128] = acc.astype(bf)
                                if lo + 128 == plo + pn:
                                    for mm_ in reversed(range(NM)):
                                        @pl.when(j == NIT - NM + mm_)
                                        def _():
                                            ocp(mm_, p).start()
            tie.finish()

        def outer(it, carry):
            lax.cond(it == 0, lambda: phase_a(it), lambda: body(it - 1))
            return carry
        lax.fori_loop(0, NIT + 1, outer, 0)

        with scope("owait"):
            for mm_ in range(NM - 1):
                for p in range(NP - ndb, NP):
                    ocp(mm_, p).wait()
            for p in range(NP):
                ocp(NM - 1, p).wait()

    def fn(x, w_gate, w_up, w_down):
        B, S, _ = x.shape
        xt = x.reshape(M, D).T
        wdt = w_down.T
        rr = max(r, 8)
        out = pl.pallas_call(
            kernel,
            in_specs=[pl.BlockSpec(memory_space=pl.ANY)] * 4,
            out_specs=pl.BlockSpec(memory_space=pl.ANY),
            out_shape=jax.ShapeDtypeStruct((D, M), x.dtype),
            scratch_shapes=[pltpu.VMEM((D, M), bf), pltpu.VMEM((M // TM, 5, TM // 2, 128), u32),
                            pltpu.VMEM((D, FA), bf), pltpu.VMEM((D, FA), bf), pltpu.VMEM((D, FA), bf),
                            pltpu.VMEM((NF, D, FB), bf), pltpu.VMEM((NF, D, FB), bf), pltpu.VMEM((NF, D, FB), bf),
                            pltpu.VMEM((NM, D, MH), f32),
                            pltpu.VMEM((2, NF, KT, FB), f32),
                            pltpu.VMEM((M // TM, KT, rr, 128), f32),
                            pltpu.VMEM((NQ, TM, 128), f32),
                            pltpu.VMEM((2, TM, 128), f32), pltpu.VMEM((NTB, TM // 2, 128), u32),
                            pltpu.VMEM((NTB, D // 2, 128), u32),
                            pltpu.VMEM((M // TM, NTA, TM // 2, 128), u32)]
                           + [pltpu.VMEM((NM, D, n) if p >= NP - ndb else (D, n), bf)
                              for p, (_, n) in enumerate(pieces)]
                           + [pltpu.SemaphoreType.DMA((7,)), pltpu.SemaphoreType.DMA((2,))],
            compiler_params=pltpu.CompilerParams(
                vmem_limit_bytes=vmem * 1024 * 1024,
            ),
        )(xt, w_gate, w_up, wdt)
        return out.T.reshape(B, S, D)
    return fn


_impl = build()


@jax.jit
def pallas_standalone__geglu_ffn__prompt_kernel(
    x: jax.Array,
    w_gate: jax.Array,
    w_up: jax.Array,
    w_down: jax.Array,
):
    return _impl(x, w_gate, w_up, w_down)
```

```python
import contextlib
import jax
import jax.numpy as jnp
from jax import lax
import jax.experimental.pallas as pl
import jax.experimental.pallas.tpu as pltpu

C0 = 0.7978845608028654
C1 = C0 * 0.044715


def _geglu2(g, u):
    z = g * (C0 + C1 * (g * g))
    p = g * u
    return p + p * jnp.tanh(z)


def build(vmem=110, scopes=0, r=160, R=32, lead=8, wt=46, wg_=50, wu_=36, wd_=51, wd4=51, front=0.985,
          lk=4, omode=0, a_front=0.9, a_gs=0.3, a3lo=0.15, tsk=2, dsk=2, tree=2, rlo=128, nhi=18, x3=1.5, snap=2, wout=4):
    D, F, M = 576, 4608, 2048
    KM, KT = 512, 64
    TM = 512
    FA, NF, MH = 384, 3, 1024
    NM = M // MH
    TPH = MH // TM
    FB = (F - FA) // NF
    NTA = FA // 128
    NTB = FB // 128
    NQ = TPH * NTB * 2
    ndb = 1
    NL = (lead + 1) // 2
    RM = TM - r
    NN = TPH * NTB
    r_of = [r if (i + 1) * nhi // NN > i * nhi // NN else min(rlo, r) for i in range(NN)]
    dn_nt = (((1,), (1,)), ((), ()))
    scope = jax.named_scope if scopes else (lambda n: contextlib.nullcontext())
    f32 = jnp.float32
    bf = jnp.bfloat16
    u32 = jnp.uint32
    psz = [TM] * (TPH - 1) + [128] * (TM // 128)
    pieces = [(sum(psz[:i]), psz[i]) for i in range(len(psz))]
    NP = len(pieces)
    NIT = NM * NF
    NSUB = MH // 128
    CH = [(0, 3), (3, 4), (7, 4)]
    assert r % 16 == 0 and R % 32 == 0

    def kernel(xt_hbm, wg_hbm, wu_hbm, wdt_hbm, o_hbm,
               xt_s, xs, wga, wua, wda, wgb, wub, wdb, acc_s, w32, xb_s, t_s, g_s, h_s, wdp, ha_s, *rest):
        o_s, sem, osem = rest

        def cp(src, dst, lo, n, s):
            return pltpu.make_async_copy(src.at[:, pl.ds(lo, n)], dst.at[:, pl.ds(lo, n)], sem.at[s])

        def cpr(src, dst, f, r0, nr, s, c0=0, nc=FB):
            return pltpu.make_async_copy(src.at[pl.ds(r0, nr), pl.ds(FA + f * FB + c0, nc)],
                                         dst.at[f, pl.ds(r0, nr), pl.ds(c0, nc)], sem.at[s])

        def wb(f, s):
            return [cpr(wg_hbm, wgb, f, 0, KM, s), cpr(wu_hbm, wub, f, 0, KM, s), cpr(wdt_hbm, wdb, f, 0, D, s)]

        def gua(c, s):
            return [cp(wg_hbm, wga, c * 128, 128, s), cp(wu_hbm, wua, c * 128, 128, s)]

        groups = [
            [cp(xt_hbm, xt_s, 0, 256, 0)],
            gua(0, 1),
            gua(1, 2) + [cp(xt_hbm, xt_s, 256, 256, 2)],
            gua(2, 3) + [cp(xt_hbm, xt_s, TM, TM, 3)]
            + [cpr(s_, d_, 0, KM, KT, 3, 0, NL * 128) for s_, d_ in ((wg_hbm, wgb), (wu_hbm, wub))],
            [cp(wdt_hbm, wda, 0, FA, 4), cp(xt_hbm, xt_s, 2 * TM, 2 * TM, 4)]
            + [cpr(s_, d_, 0, KM, KT, 4, NL * 128, FB - NL * 128) for s_, d_ in ((wg_hbm, wgb), (wu_hbm, wub))]
            + [cpr(s_, d_, f, KM, KT, 4) for f in range(1, NF) for s_, d_ in ((wg_hbm, wgb), (wu_hbm, wub))],
            wb(0, 5),
            [c for f in range(1, NF) for c in wb(f, 6)],
        ]

        def wait(g):
            for c in groups[g]:
                c.wait()

        for g in groups:
            for c in g:
                c.start()

        def mm(a, b):
            return jnp.dot(a, b, preferred_element_type=f32)

        def down(wd, h):
            return lax.dot_general(wd, h, dn_nt, preferred_element_type=f32)

        def xpose(lo, n):
            x = xt_s[:, lo:lo + n].T
            t, r0 = lo // TM, (lo % TM) // 2
            for kt in range(4):
                xs[t, kt, r0:r0 + n // 2, :] = pltpu.bitcast(x[:, kt * 128:(kt + 1) * 128], u32)
            xs[t, 4, r0:r0 + n // 2, :] = jnp.concatenate(
                [pltpu.bitcast(x[:, KM:D], u32), jnp.zeros((n // 2, 128 - KT), u32)], axis=1)
            return x

        def xmain(tt):
            return jnp.concatenate([pltpu.bitcast(xs[tt, kt], bf) for kt in range(4)], axis=1)

        def xtail(tt, a, n):
            return pltpu.bitcast(xs[tt, 4, a // 2:(a + n) // 2, 0:KT], bf)

        class Ties:
            def __init__(self, it, jobs, total_w, front):
                self.it, self.masks = it, {}
                self.jobs, self.W, self.front = jobs, total_w, front
                self.total = sum(r_of[jb[4] // 2] // 8 * KT for jb in jobs)
                self.w = 0.0
                self.done = self.i = self.r0 = self.k = 0
                self.acc = None
                self.lumps = []
                self.scale = 1.0
                self.wm = 0.0
                self.Wm = total_w

            def mask(self, rows):
                if rows not in self.masks:
                    self.masks[rows] = lax.broadcasted_iota(jnp.int32, (rows, 128), 1) < (self.it - 1000)
                return self.masks[rows]

            def skip(self, w):
                self.w += w
                self.wm += w * self.scale

            def __call__(self, piece, w):
                self.skip(w)
                if self.lumps and self.w >= self.lumps[0][0] * self.W:
                    self.lumps.pop(0)[1](piece)
                target = min(self.total, int(self.total * self.wm / (self.Wm * self.front)))
                while target > self.done:
                    tile, f, which, n, slot = self.jobs[self.i]
                    rj = r_of[slot // 2]
                    nr = min(R, rj - self.r0)
                    kk = min(-((self.done - target) // (nr // 8)), KT - self.k)
                    if KT - self.k - kk <= snap:
                        kk = KT - self.k
                    cs = pl.ds(n * 128, 128)
                    ps = [xb_s[tile, k, pl.ds(r - rj + self.r0, nr), :] * w32[which, f, pl.ds(k, 1), cs]
                          for k in range(self.k, self.k + kk)]
                    chains = [None] * tree
                    chains[0] = self.acc
                    for i, p in enumerate(ps):
                        c = i % tree
                        chains[c] = p if chains[c] is None else chains[c] + p
                    chains = [c for c in chains if c is not None]
                    acc = chains[0]
                    for c in chains[1:]:
                        acc = acc + c
                    self.done += kk * (nr // 8)
                    self.k += kk
                    self.acc = acc
                    pc = piece if nr == R else piece[0:nr]
                    if self.k < KT:
                        pc = jnp.where(self.mask(nr), acc, pc)
                        return pc if nr == R else jnp.concatenate([pc, piece[nr:]], axis=0)
                    t_s[slot, pl.ds(TM - rj + self.r0, nr), :] = jnp.where(self.mask(nr), pc, acc)
                    self.k, self.acc = 0, None
                    self.r0 += nr
                    if self.r0 == rj:
                        self.r0 = 0
                        self.i += 1
                    if target - self.done <= snap * (R // 8):
                        break
                return piece

            def all(self, res, w_per_beat):
                outs = [self(res[a:a + R], w_per_beat * (R // 16)) for a in range(0, res.shape[0] - R + 1, R)]
                rem = res.shape[0] % R
                if rem:
                    self.skip(w_per_beat * (rem // 16))
                    outs.append(res[res.shape[0] - rem:])
                return jnp.concatenate(outs, axis=0) if len(outs) > 1 else outs[0]

            def finish(self):
                assert self.done == self.total and not self.lumps, (self.done, self.total, len(self.lumps))

        def ntile(tie, tt, q, wg, wu, rm, h_dst, par, ready=None):
            H = -(-rm // 32) * 16
            parts = [(0, 0, H), (0, H, rm - H), (1, 0, rm - H), (1, rm - H, H)]
            res = [mm(xtail(tt, a0, n_), (wg, wu)[w_](KM, D)) for w_, a0, n_ in parts]
            for a in range(0, H, R):
                for pi, ((w_, a0, nrows), rs_) in enumerate(zip(parts, res)):
                    n_ = min(R, nrows - a)
                    if n_ <= 0:
                        continue
                    v = rs_[a:a + n_]
                    if n_ == R and (pi + 1) % tsk == 0:
                        v = tie(v, wt * (R // 16) / 4)
                    else:
                        tie.skip(wt * (n_ // 16) / 4)
                    t_s[q + w_, pl.ds(a0 + a, n_), :] = v
            gmain = mm(xmain(tt), wg(0, KM))
            g_s[par, 0:rm] = tie.all(gmain[0:rm] + t_s[q, 0:rm], wg_)
            if rm < TM:
                assert ready(q)
                g_s[par, rm:TM] = tie.all(gmain[rm:TM] + t_s[q, rm:TM], wg_)
            umain = mm(xmain(tt), wu(0, KM))
            u = tie.all(umain[0:rm] + t_s[q + 1, 0:rm], wu_)
            if rm < TM:
                assert ready(q + 1)
                u1 = tie.all(umain[rm:TM] + t_s[q + 1, rm:TM], wu_)
                u = jnp.concatenate([u, u1], axis=0)
            h_dst[...] = _geglu2(g_s[par], u).astype(bf)

        def down3(tie, wdf, hf, acc_ref, first, fresh=False):
            cat = lambda xs_: jnp.concatenate(xs_, axis=1) if len(xs_) > 1 else xs_[0]
            seen = set()
            for ri, rnd in enumerate((((0, (0, 1, 2)), (1, (0,))), ((1, (1, 2)), (2, (0, 1))),
                                      ((2, (2,)), (3, (0, 1, 2))))):
                wq = wd4 - (3 if (fresh and ri == 0) else 0)
                ps = [down(cat([wdf(n) for n in ks]), cat([hf(n, a) for n in ks])) for a, ks in rnd]
                for r0 in range(0, D, R):
                    rr_ = min(R, D - r0)
                    for pi, ((a, ks), p_) in enumerate(zip(rnd, ps)):
                        v = p_[r0:r0 + rr_]
                        if not (first and a not in seen):
                            v = acc_ref[r0:r0 + rr_, a * 128:(a + 1) * 128] + v
                        if rr_ == R and (pi + 1) % dsk == 0:
                            v = tie(v, wq * (R // 16) / 2)
                        else:
                            tie.skip(wq * (rr_ // 16) / 2)
                        acc_ref[r0:r0 + rr_, a * 128:(a + 1) * 128] = v
                seen.update(a for a, _ in rnd)

        w_nt = lambda rm: wt * (rm / 32) + (wg_ + wu_) * (TM // 16)
        w_d4 = wd4 * (D // 16)

        def w_dsub(t, ci, a):
            return wd_ - (4 if (t == 0 and a == 0) else 0) - (wout if ci == len(CH) - 1 else 0)

        def xb_lump(tie, t, g0, k0):
            def emit(piece):
                n_ = min(R, r // 2 - g0)
                src = xs[t, 4, pl.ds(RM // 2 + g0, n_), :]
                src = jnp.where(tie.mask(n_), pltpu.bitcast(piece[0:n_], u32), src)
                for k in range(k0, k0 + lk):
                    b = jnp.broadcast_to(src[:, k:k + 1], (n_, 128))
                    xb_s[t, k, pl.ds(2 * g0, 2 * n_), :] = pltpu.bitcast(b, bf).astype(f32)
            return emit

        def xb_lumps(tie, t):
            return [xb_lump(tie, t, g0, k0) for k0 in range(0, KT, lk) for g0 in range(0, r // 2, R)]

        def w32_lump(tie, f, which, n):
            def emit(piece):
                cs = pl.ds(n * 128, 128)
                src = pltpu.bitcast((wgb, wub)[which][f, KM:D, cs], u32)
                src = jnp.where(tie.mask(KT // 2), pltpu.bitcast(piece[0:KT // 2], u32), src)
                w32[which, f, :, cs] = pltpu.bitcast(src, bf).astype(f32)
            return emit

        def spread(ls, a, b):
            return [(a + (b - a) * i / len(ls), l) for i, l in enumerate(ls)]

        def tail_job(q, m, f):
            t, n, which = q // (2 * NTB), (q % (2 * NTB)) // 2, q % 2
            return (m * TPH + t, f, which, n, q)

        def phase_a(it):
            def gu_v(x, lo, n, rr, t, r0):
                wg, wu = wga[:, lo:lo + n], wua[:, lo:lo + n]
                for a in range(0, x.shape[0], rr):
                    h = _geglu2(mm(x[a:a + rr], wg), mm(x[a:a + rr], wu)).astype(bf)
                    for c in range(n // 128):
                        ha_s[t, lo // 128 + c, r0 + a:r0 + a + rr, :] = h[:, c * 128:(c + 1) * 128]

            def nt_a(tie, tt, n, cnt):
                cs = pl.ds(n * 128, 128)
                ntile(tie, tt, NQ - 4 + 2 * (cnt % 2), lambda a, b: wga[a:b, cs], lambda a, b: wua[a:b, cs],
                      TM, ha_s.at[tt, n], cnt % 2)

            def dn_a(tie, tt):
                accv = acc_s.at[tt // TPH, :, (tt % TPH) * TM:(tt % TPH + 1) * TM]
                if tt == 0:
                    for n in range(NTA):
                        wdp[n] = pltpu.bitcast(wda[:, n * 128:(n + 1) * 128], u32)
                down3(tie, lambda n: pltpu.bitcast(wdp[n], bf),
                      lambda n, a: ha_s[tt, n, a * 128:(a + 1) * 128, :], accv, True)

            with scope("w0"):
                wait(0)
            xa = xpose(0, 256)
            with scope("w1"):
                wait(1)
            with scope("s1"):
                gu_v(xa, 0, 128, 128, 0, 0)
            with scope("w2"):
                wait(2)
            with scope("s2"):
                xb = xpose(256, 256)
                gu_v(xa, 128, 128, 128, 0, 0)
                gu_v(xb, 0, 256, 256, 0, 256)
            with scope("w3"):
                wait(3)
            with scope("s3"):
                tie = Ties(it, [], 4 * w_nt(TM), 1.0)
                if r:
                    l0 = [w32_lump(tie, 0, which, n) for n in range(NL) for which in range(2)]
                    lx = xb_lumps(tie, 0) + xb_lumps(tie, 1)
                    n3 = int(len(lx) * x3 / 2)
                    tie.lumps = spread(l0, 0.02, a3lo) + spread(lx[:n3], a3lo, 0.95)
                xpose(TM, TM)
                nt_a(tie, 0, 2, 0)
                for n in range(NTA):
                    nt_a(tie, 1, n, n + 1)
                tie.finish()
            with scope("w4"):
                wait(4)
            with scope("s4"):
                jobs = [tail_job(q, 0, 0) for q in range(lead)] if r else []
                tie = Ties(it, jobs, 2 * NTA * w_nt(TM) + 4 * NTA * w_d4, a_front)
                if r:
                    l1 = [w32_lump(tie, f, which, n) for f in range(NF) for n in range(NTB) for which in range(2)
                          if not (f == 0 and n < NL)]
                    lx = (xb_lumps(tie, 0) + xb_lumps(tie, 1))[n3:] + xb_lumps(tie, 2) + xb_lumps(tie, 3)
                    fd = 2 * NTA * w_d4 / tie.W
                    tie.lumps = spread(lx, fd, 1 - fd - 0.01) + spread(l1, 1 - fd, 0.98)
                    tie.Wm = 2 * NTA * w_nt(TM) * a_gs + 4 * NTA * w_d4
                xpose(2 * TM, TM)
                dn_a(tie, 0)
                xpose(3 * TM, TM)
                dn_a(tie, 1)
                tie.scale = a_gs
                for tt in (2, 3):
                    for n in range(NTA):
                        nt_a(tie, tt, n, tt * NTA + n)
                tie.scale = 1.0
                dn_a(tie, 2)
                dn_a(tie, 3)
                tie.finish()
            with scope("w5"):
                wait(5)

        def ocp(mm_, p):
            return pltpu.make_async_copy(o_s.at[mm_, p], o_hbm.at[:, pl.ds(mm_ * MH + p * 128, 128)], osem.at[0])

        def body(j):
            f = lax.shift_right_logical(j, 1)
            m = lax.bitwise_and(j, 1)
            jn = jnp.minimum(j + 1, NIT - 1)
            fn_ = lax.shift_right_logical(jn, 1)
            mn = lax.bitwise_and(jn, 1)

            @pl.when(j == 1)
            def _():
                wait(6)

            jobs = ([tail_job(q, m, f) for q in range(lead, NQ)] + [tail_job(q, mn, fn_) for q in range(lead)]) \
                if r else []
            W = sum(w_nt(TM - rr_) for rr_ in r_of) - 3 * (D // 16) + sum(
                sum(w_dsub(t, ci, a) * (D // 16) for a in range(4)) if nn == 4 else nn * w_d4
                for t in range(TPH) for ci, (_, nn) in enumerate(CH))
            tie = Ties(j, jobs, W, front)
            ready = lambda q: q < lead + tie.i

            with scope("body"):
                for t in range(TPH):
                    tt = m * TPH + t
                    accv = acc_s.at[m, :, t * TM:(t + 1) * TM]
                    for ci, (n0, nn) in enumerate(CH):
                        for n in range(n0, n0 + nn):
                            cs = pl.ds(n * 128, 128)
                            ntile(tie, tt, (t * NTB + n) * 2, lambda a, b: wgb[f, a:b, cs],
                                  lambda a, b: wub[f, a:b, cs], TM - r_of[t * NTB + n], h_s.at[n], n % 2, ready)
                        if nn != 4:
                            packed = set()

                            def wdf(n):
                                if t == 0 and n not in packed:
                                    packed.add(n)
                                    wd = wdb[f, :, (n0 + n) * 128:(n0 + n + 1) * 128]
                                    wdp[n0 + n] = pltpu.bitcast(wd, u32)
                                    return wd
                                return pltpu.bitcast(wdp[n0 + n], bf)
                            down3(tie, wdf, lambda n, a: h_s[n0 + n, a * 128:(a + 1) * 128, :],
                                  accv, False, t == 0)
                            continue
                        for a in range(TM // 128):
                            if t == 0 and a == 0:
                                wd = wdb[f, :, n0 * 128:(n0 + nn) * 128]
                                for n in range(nn):
                                    wdp[n0 + n] = pltpu.bitcast(wd[:, n * 128:(n + 1) * 128], u32)
                            else:
                                wd = jnp.concatenate([pltpu.bitcast(wdp[n], bf) for n in range(n0, n0 + nn)], axis=1)
                            h = jnp.concatenate([h_s[n, a * 128:(a + 1) * 128, :]
                                                 for n in range(n0, n0 + nn)], axis=1)
                            lo = t * TM + a * 128
                            acc = tie.all(accv[:, a * 128:(a + 1) * 128] + down(wd, h), w_dsub(t, ci, a))
                            accv[:, a * 128:(a + 1) * 128] = acc
                            if ci == len(CH) - 1:
                                p = lo // 128
                                o_s[m, p] = (0.5 * acc).astype(bf)
                                for mm_ in reversed(range(NM)):
                                    @pl.when(j == NIT - NM + mm_)
                                    def _():
                                        ocp(mm_, p).start()
                                if a == TM // 128 - 1 and t < TPH - 1:
                                    def pin(piece):
                                        o_s[m, NSUB, 0:16, :] = piece[0:16].astype(bf)
                                    tie.lumps.append((0.0, pin))
            tie.finish()

        def outer(it, carry):
            lax.cond(it == 0, lambda: phase_a(it), lambda: body(it - 1))
            return carry
        lax.fori_loop(0, NIT + 1, outer, 0)

        with scope("owait"):
            for mm_ in range(NM):
                for p in range(NSUB):
                    ocp(mm_, p).wait()

    def fn(x, w_gate, w_up, w_down):
        B, S, _ = x.shape
        xt = x.reshape(M, D).T
        wdt = w_down.T
        rr = max(r, 8)
        out = pl.pallas_call(
            kernel,
            in_specs=[pl.BlockSpec(memory_space=pl.ANY)] * 4,
            out_specs=pl.BlockSpec(memory_space=pl.ANY),
            out_shape=jax.ShapeDtypeStruct((D, M), x.dtype),
            scratch_shapes=[pltpu.VMEM((D, M), bf), pltpu.VMEM((M // TM, 5, TM // 2, 128), u32),
                            pltpu.VMEM((D, FA), bf), pltpu.VMEM((D, FA), bf), pltpu.VMEM((D, FA), bf),
                            pltpu.VMEM((NF, D, FB), bf), pltpu.VMEM((NF, D, FB), bf), pltpu.VMEM((NF, D, FB), bf),
                            pltpu.VMEM((NM, D, MH), f32),
                            pltpu.VMEM((2, NF, KT, FB), f32),
                            pltpu.VMEM((M // TM, KT, rr, 128), f32),
                            pltpu.VMEM((NQ, TM, 128), f32),
                            pltpu.VMEM((2, TM, 128), f32), pltpu.VMEM((NTB, TM, 128), bf),
                            pltpu.VMEM((NTB, D // 2, 128), u32),
                            pltpu.VMEM((M // TM, NTA, TM, 128), bf)]
                           + [pltpu.VMEM((NM, NSUB + 1, D, 128), bf)]
                           + [pltpu.SemaphoreType.DMA((7,)), pltpu.SemaphoreType.DMA((1,))],
            compiler_params=pltpu.CompilerParams(
                vmem_limit_bytes=vmem * 1024 * 1024,
            ),
        )(xt, w_gate, w_up, wdt)
        return out.T.reshape(B, S, D)
    return fn


_impl = build()


@jax.jit
def pallas_standalone__geglu_ffn__prompt_kernel(
    x: jax.Array,
    w_gate: jax.Array,
    w_up: jax.Array,
    w_down: jax.Array,
):
    return _impl(x, w_gate, w_up, w_down)
```

```python
import contextlib
import jax
import jax.numpy as jnp
from jax import lax
import jax.experimental.pallas as pl
import jax.experimental.pallas.tpu as pltpu

C0 = 0.7978845608028654
C1 = C0 * 0.044715


def _geglu2(g, u):
    z = g * (C0 + C1 * (g * g))
    p = g * u
    return p + p * jnp.tanh(z)


def build(vmem=120, scopes=0, rt=320, lead=5, hb1=27, hb2=41, hb3=6, wt=58, wg_=52, wu_=36, wd_=50, tsk=2,
          fr_g=0.997, fr_d=0.98, wk=16, hbc=1, w1=8, w2=6, w3=4, x2=1, x3=2, m1=13, m2=8, m3=13,
          vt=0.2, lo_=0.02, hi_=0.93, nosc=1, wbr=0, uq_=1.0, nq_=4, osp=384):
    D, F, M = 576, 4608, 2048
    KM, KT, KH = 512, 64, 32
    TA = 512
    FA, NF, MH = 384, 3, 1024
    R = 32
    NM = M // MH
    NT = M // TA
    NS = MH // 128
    FB = (F - FA) // NF
    NTA = FA // 128
    NTB = FB // 128
    NQ = NTB * 2
    NBLK = rt // R
    HBQ = 2 * NBLK
    NHB = NQ * HBQ
    dn_nt = (((1,), (1,)), ((), ()))
    scope = jax.named_scope if scopes else (lambda n: contextlib.nullcontext())
    f32, bf, u32, i32 = jnp.float32, jnp.bfloat16, jnp.uint32, jnp.int32
    NIT = NM * NF
    NE = 4
    NC = NF * NTB
    assert rt % 32 == 0 and NBLK <= 10 and (lead + 1) // 2 <= NE

    def kernel(xt_hbm, wg_hbm, wu_hbm, wdt_hbm, o_hbm,
               xt_s, xs, wga, wua, wda, wgb, wub, wdb, acc_s, wb_s, xb_s, tm_s, tv_s, g_s, j_s, h_s, ha_s,
               wdp, o_s, sem, osem):

        def cp(src, dst, lo, n, s):
            return pltpu.make_async_copy(src.at[:, pl.ds(lo, n)], dst.at[:, pl.ds(lo, n)], sem.at[s])

        def cpr(src, dst, f, r0, nr, s, c0=0, nc=FB):
            return pltpu.make_async_copy(src.at[pl.ds(r0, nr), pl.ds(FA + f * FB + c0, nc)],
                                         dst.at[f, pl.ds(r0, nr), pl.ds(c0, nc)], sem.at[s])

        def wb(f, s):
            return [cpr(wg_hbm, wgb, f, 0, KM, s), cpr(wu_hbm, wub, f, 0, KM, s), cpr(wdt_hbm, wdb, f, 0, D, s)]

        def gua(c, s):
            return [cp(wg_hbm, wga, c * 128, 128, s), cp(wu_hbm, wua, c * 128, 128, s)]

        gw = ((wg_hbm, wgb), (wu_hbm, wub))
        groups = [
            [cp(xt_hbm, xt_s, 0, 256, 0)],
            gua(0, 1),
            gua(1, 2) + [cp(xt_hbm, xt_s, 256, 256, 2)],
            gua(2, 3) + [cp(xt_hbm, xt_s, TA, TA, 3)] + [cpr(s_, d_, 0, KM, KT, 3, 0, NE * 128) for s_, d_ in gw],
            [cp(wdt_hbm, wda, 0, FA, 4), cp(xt_hbm, xt_s, 2 * TA, 2 * TA, 4)]
            + [cpr(s_, d_, 0, KM, KT, 4, NE * 128, FB - NE * 128) for s_, d_ in gw]
            + [cpr(s_, d_, f, KM, KT, 4) for f in range(1, NF) for s_, d_ in gw],
            wb(0, 5),
            [c for f in range(1, NF) for c in wb(f, 6)],
        ]

        def wait(g):
            for c in groups[g]:
                c.wait()

        for g in groups:
            for c in g:
                c.start()

        def mm(a, b):
            return jnp.dot(a, b, preferred_element_type=f32)

        def down(wd, h):
            return lax.dot_general(wd, h, dn_nt, preferred_element_type=f32)

        def lanes(n, w=128):
            return pl.ds(pl.multiple_of(n * w, w), w)

        def uloop(lo, hi, fn):
            lax.fori_loop(lo, hi, lambda i, c: (fn(i), c)[1], 0, unroll=True)

        def xpose(lo, n):
            x = xt_s[:, lo:lo + n].T
            m, r0 = lo // MH, (lo % MH) // 2
            for kt in range(4):
                xs[m, kt, r0:r0 + n // 2, :] = pltpu.bitcast(x[:, kt * 128:(kt + 1) * 128], u32)
            xs[m, 4, r0:r0 + n // 2, :] = jnp.concatenate(
                [pltpu.bitcast(x[:, KM:D], u32), jnp.zeros((n // 2, 128 - KT), u32)], axis=1)
            return x

        class Ties:
            def __init__(self, it, hb0, nhb, cur, nxt, total_w, front, lumps=(), total_v=None):
                self.it, self.masks = it, {}
                self.hb0, self.cur, self.nxt = hb0, cur, nxt
                self.total = nhb * KH
                self.W = total_w * front
                self.w = self.v = 0.0
                self.done = self.k = 0
                self.acc = self.job = None
                self.lumps = [((total_v or total_w) * (lo_ + (hi_ - lo_) * i / len(lumps)), l)
                              for i, l in enumerate(lumps)]

            def mask(self, rows=R):
                if rows not in self.masks:
                    self.masks[rows] = lax.broadcasted_iota(i32, (rows, 128), 1) < (self.it - 1000)
                return self.masks[rows]

            def decode(self, i):
                b = self.hb0 + i
                m, f = self.cur
                if self.nxt is not None:
                    wrap = b >= NHB
                    b = lax.rem(b, NHB)
                    m, f = lax.select(wrap, self.nxt[0], m), lax.select(wrap, self.nxt[1], f)
                q, e = lax.div(b, HBQ), lax.rem(b, HBQ)
                return q, lax.rem(e, 2), lax.div(e, 2), m, f

            def skip(self, w, v=None):
                self.w += w
                self.v += w if v is None else v

            def __call__(self, piece, slot, w, v=None):
                self.skip(w, v)
                if self.lumps and self.v >= self.lumps[0][0]:
                    self.lumps.pop(0)[1](lambda x: lax.select(
                        self.mask(x.shape[0]), pltpu.bitcast(piece()[0:x.shape[0]], u32), x))
                target = min(self.total, int(self.total * self.w / self.W))
                while target > self.done:
                    if self.job is None:
                        self.job = self.decode(self.done // KH)
                    q, half, blk, m, f = self.job
                    kk = min(target - self.done, KH - self.k)
                    if KH - self.k - kk <= 2:
                        kk = KH - self.k
                    ks = pl.ds(half * KH + self.k, kk)
                    p = xb_s[m, blk, ks] * wb_s[f, q, ks]
                    h2 = (kk + 1) // 2
                    acc = jnp.sum(p[0:h2], axis=0)
                    if self.acc is not None:
                        acc = acc + self.acc
                    if kk > h2:
                        acc = acc + jnp.sum(p[h2:kk], axis=0)
                    self.done += kk
                    self.k += kk
                    self.acc = acc
                    a2 = acc.reshape(R, 128)
                    if self.k < KH:
                        slot[...] = a2
                        return
                    tv_s[q, half, lanes(blk, R), :] = lax.select(self.mask(), piece(), a2)
                    self.k, self.acc, self.job = 0, None, None
                    if target - self.done <= 2:
                        break

            def store(self, dst, val, w_per_beat, quiet=1.0):
                for a in range(0, val.shape[0], R):
                    qf = quiet if a >= val.shape[0] - nq_ * R else 1.0
                    self(lambda: val[a:a + R], dst.at[pl.ds(a, R), :], w_per_beat * 2 * qf, 2.0)
                dst[...] = val

            def finish(self):
                assert self.done == self.total and not self.lumps, (self.done, self.total, len(self.lumps))

        w_gu = lambda tm, rv: wt * ((tm - rv) / 32) + (wg_ + wu_) * (tm // 16) - (1 - uq_) * wu_ * 2 * nq_
        v_gu = lambda tm, rv: vt * ((tm - rv) / 32) + 2 * (tm // 16)

        def gu_unit(tie, xr, tm, rv, q, wg, wu, h_dst, mid=None):
            H = (tm - rv) // 2
            parts = [(0, rv), (0, rv + H), (1, rv), (1, rv + H)]
            res = [mm(pltpu.bitcast(xr(4, a0, H)[:, 0:KT], bf), (wg, wu)[w_](KM, D)) for w_, a0 in parts]
            for a in range(0, H, R):
                n_ = min(R, H - a)
                for pi, ((w_, a0), rs_) in enumerate(zip(parts, res)):
                    if n_ == R and (pi + 1) % tsk == 0:
                        tie(lambda: rs_[a:a + R], tm_s.at[w_, pl.ds(a0 + a, R), :], wt * (n_ // 16) / 4,
                            vt * (n_ // 16) / 4)
                    else:
                        tie.skip(wt * (n_ // 16) / 4, vt * (n_ // 16) / 4)
            for (w_, a0), rs_ in zip(parts, res):
                tm_s[w_, a0:a0 + H, :] = rs_

            def full(w_):
                xmain = jnp.concatenate([pltpu.bitcast(xr(kt, 0, tm), bf) for kt in range(4)], axis=1)
                main = mm(xmain, (wg, wu)[w_](0, KM))
                if not rv:
                    return main + tm_s[w_, 0:tm]
                return jnp.concatenate([(main[0:rv] + tv_s[q + w_, 0]) + tv_s[q + w_, 1],
                                        main[rv:tm] + tm_s[w_, rv:tm]], axis=0)
            tie.store(g_s.at[0:tm], full(0), wg_)
            if mid is not None:
                mid()
            u = full(1)
            tie.store(j_s.at[0:tm], u, wu_, uq_)
            h_dst[...] = _geglu2(g_s[0:tm], u).astype(bf)
            tie.finish()

        def dn_unit(tie, wd, h, m):
            for t in range(MH // 512):
                p_ = down(wd(), h(t))
                for a in range(3):
                    acc_s[m, 4 * t + a] += p_[:, a * 128:(a + 1) * 128]
                dst = acc_s.at[m, 4 * t + 3]
                tie.store(dst, dst[...] + p_[:, 384:512], wd_)

        def d3_unit(tie, tt):
            cat = lambda xs_: jnp.concatenate(xs_, axis=1) if len(xs_) > 1 else xs_[0]
            m, a0 = lax.div(tt, 2), lax.rem(tt, 2) * 4
            seen = set()
            for rnd in (((0, (0, 1, 2)), (1, (0,))), ((1, (1, 2)), (2, (0, 1))), ((2, (2,)), (3, (0, 1, 2)))):
                vs = []
                for a, ks in rnd:
                    v = down(wda[:, ks[0] * 128:(ks[-1] + 1) * 128],
                             cat([ha_s[tt * NTA + n, a * 128:(a + 1) * 128, :] for n in ks]))
                    dst = acc_s.at[m, a0 + a]
                    vs.append((dst, dst[...] + v if a in seen else v))
                for r0 in range(0, D, R):
                    for dst, v in vs:
                        tie(lambda: v[r0:r0 + R], dst.at[pl.ds(r0, R), :], 1.0)
                for dst, v in vs:
                    dst[...] = v
                seen.update(a for a, _ in rnd)
            tie.finish()

        def xb_lump(m, blk, k0, nk):
            def emit(pin):
                src = pin(xs[m, 4, lanes(blk, 16), :])
                b = jnp.stack([jnp.broadcast_to(src[:, k:k + 1], (16, 128)) for k in range(k0, k0 + nk)])
                xb_s[m, blk, k0:k0 + nk] = pltpu.bitcast(b, bf).astype(f32).reshape(nk, 4, 8, 128)
            return emit

        def wb_lump(c, which, k0, nk):
            def emit(pin):
                f, n = lax.div(c, NTB), lax.rem(c, NTB)
                src = pin(pltpu.bitcast((wgb, wub)[which][f, KM + k0:KM + k0 + nk, lanes(n)], u32))
                v = pltpu.bitcast(src, bf).astype(f32)
                if wbr:
                    v = jnp.broadcast_to(v.reshape(nk, 1, 128), (nk, 8, 128))
                else:
                    v = jnp.stack([jnp.broadcast_to(v[k:k + 1], (8, 128)) for k in range(nk)])
                wb_s[f, 2 * n + which, k0:k0 + nk, 0] = v
            return emit

        def wb_lumps(c, which):
            return [wb_lump(c, which, k0, wk) for k0 in range(0, KT, wk)]

        def phase_a(it):
            zero = jnp.zeros((), i32)

            def gu_v(x, lo, n, rr, r0):
                wg, wu = wga[:, lo:lo + n], wua[:, lo:lo + n]
                for a in range(0, x.shape[0], rr):
                    h = _geglu2(mm(x[a:a + rr], wg), mm(x[a:a + rr], wu)).astype(bf)
                    for c in range(n // 128):
                        ha_s[lo // 128 + c, r0 + a:r0 + a + rr, :] = h[:, c * 128:(c + 1) * 128]

            def mix(a, b):
                out = [(i / len(a), x) for i, x in enumerate(a)] + [((i + .5) / len(b), x) for i, x in enumerate(b)]
                return [x for _, x in sorted(out, key=lambda e: e[0])]

            def xl_at(m, blk0, nb):
                return [xb_lump(m, jnp.minimum(blk0 + i, NBLK - 1), k0, 8) for i in range(nb) for k0 in range(0, KT, 8)]

            def wl_at(i0, n):
                return [l for i in range(n) for l in wb_lumps(jnp.minimum(NE + i0 + i // 2, NC - 1), i % 2)]

            def gu_a(u, m, lumps, hb0=0, nhb=0):
                cs, tt = lanes(lax.rem(u, NTA)), lax.div(u, NTA)
                tie = Ties(it, hb0, nhb, (zero, zero), None, w_gu(TA, 0), fr_d, lumps, v_gu(TA, 0))
                row0 = lax.rem(tt, 2) * (TA // 2)
                xr = lambda kt, a, n: xs[m, kt, pl.ds(pl.multiple_of(row0 + a // 2, 8), n // 2), :]
                gu_unit(tie, xr, TA, 0, 0, lambda a, b: wga[a:b, cs], lambda a, b: wua[a:b, cs], ha_s.at[u])

            def d3_a(tt, lumps, hb0, nhb):
                tie = Ties(it, hb0, nhb, (zero, zero), None, 6 * (D // R), fr_d, lumps)
                d3_unit(tie, tt)

            nopin = lambda v: v
            with scope("w0"):
                wait(0)
            xa = xpose(0, 256)
            xb_lump(0, 0, 0, KT)(nopin)
            with scope("w1"):
                wait(1)
            with scope("s1"):
                gu_v(xa, 0, 128, 128, 0)
                xb_lump(0, 1, 0, KT)(nopin)
            with scope("w2"):
                wait(2)
            with scope("s2"):
                xb = xpose(256, 256)
                gu_v(xa, 128, 128, 128, 0)
                gu_v(xb, 0, 256, 256, 256)
            with scope("w3"):
                wait(3)
            with scope("s3"):
                xpose(TA, TA)
                uloop(2, 6, lambda u: gu_a(u, 0, mix(xl_at(0, 2 * u - 2, 2), wb_lumps(u - 2, 0) + wb_lumps(u - 2, 1))))
            with scope("w4"):
                wait(4)
            with scope("s4"):
                assert 2 * w1 + 6 * w2 + 2 * w3 >= 2 * (NC - NE) and 6 * x2 + 2 * x3 >= NBLK
                assert 2 * m1 + 6 * m2 + 2 * m3 >= lead * HBQ
                xpose(2 * TA, TA)
                xpose(3 * TA, TA)
                uloop(0, 2, lambda tt: d3_a(tt, wl_at(tt * (w1 // 2), w1), tt * m1, m1))
                uloop(6, 12, lambda u: gu_a(u, 1, mix(xl_at(1, (u - 6) * x2, x2), wl_at(w1 + (u - 6) * (w2 // 2), w2)),
                                            2 * m1 + (u - 6) * m2, m2))
                uloop(2, 4, lambda tt: d3_a(
                    tt, mix(xl_at(1, 6 * x2 + (tt - 2) * x3, x3), wl_at(w1 + 3 * w2 + (tt - 2) * (w3 // 2), w3)),
                    jnp.minimum(2 * m1 + 6 * m2 + (tt - 2) * m3, lead * HBQ - m3), m3))
            with scope("w5"):
                wait(5)

        OS = [(0, D)] if not osp else [(0, osp), (osp, D - osp)]

        def ocp(m_, a, i):
            rows = pl.ds(*OS[i])
            return pltpu.make_async_copy(o_s.at[m_, a, rows], o_hbm.at[rows, lanes(m_ * NS + a)], osem.at[0])

        assert 4 * hb1 + (NTB - 4) * hb2 + NS * hb3 >= NHB
        for n in range(NTB):
            assert lead * HBQ + min(n, 4) * hb1 + max(n - 4, 0) * hb2 >= (2 * n + 2) * HBQ, n
        FN = (0, 1, 2, NTB - 1)

        def body(j):
            cur = (lax.bitwise_and(j, 1), lax.shift_right_logical(j, 1))
            jn = jnp.minimum(j + 1, NIT - 1)
            nxt = (lax.bitwise_and(jn, 1), lax.shift_right_logical(jn, 1))
            m, f = cur

            @pl.when(j == 1)
            def _():
                wait(6)

            base = lead * HBQ
            if hbc:
                hu = h_s.bitcast(u32)
                hld = lambda n, i, sz: pltpu.bitcast(hu[n, lanes(i, sz // 2), :], bf)
            else:
                hld = lambda n, i, sz: h_s[n, lanes(i, sz), :]
            xr = lambda kt, a, n_: xs[m, kt, a // 2:(a + n_) // 2, :]

            def unit(n, with_d):
                cs = lanes(n)
                hb0 = base + (4 * hb1 + (n - 4) * hb2 if with_d else n * hb1)
                tie = Ties(j, hb0, hb2 if with_d else hb1, cur, nxt if with_d else None,
                           w_gu(MH, rt) + (2 * (D // 16) * wd_ if with_d else 0), fr_g)
                mid = None
                if with_d:
                    mid = lambda: dn_unit(tie, lambda: wdb[f, :, lanes(n - 1)], lambda t: hld(n - 1, t, 512), m)
                gu_unit(tie, xr, MH, rt, 2 * n, lambda a, b: wgb[f, a:b, cs], lambda a, b: wub[f, a:b, cs],
                        h_s.at[n], mid)

            def final(a):
                hb0 = jnp.minimum(base + 4 * hb1 + (NTB - 4) * hb2 + a * hb3, base + NHB - hb3)
                tie = Ties(j, hb0, hb3, cur, nxt, D // 16, fr_d)
                wd = jnp.concatenate([pltpu.bitcast(wdp[i], bf) for i in range(4)], axis=1)
                h = jnp.concatenate([hld(n, a, 128) for n in FN], axis=1)
                dst = acc_s.at[m, a]
                acc = dst[...] + down(wd, h)
                tie.store(dst, acc, 1.0)
                tie.finish()
                for i, (r0, nr) in enumerate(OS):
                    o_s[m, a, r0:r0 + nr] = (0.5 * acc[r0:r0 + nr]).astype(bf)
                    for m_ in range(NM):
                        @pl.when(j == NIT - NM + m_)
                        def _():
                            ocp(m_, a, i).start()

            with scope("body"):
                uloop(0, 4, lambda n: unit(n, False))
                uloop(4, NTB, lambda n: unit(n, True))
                for i, n in enumerate(FN):
                    wdp[i] = pltpu.bitcast(wdb[f, :, n * 128:(n + 1) * 128], u32)
                uloop(0, NS, final)

        def outer(it, carry):
            lax.cond(it == 0, lambda: phase_a(it), lambda: body(it - 1))
            return carry
        lax.fori_loop(0, NIT + 1, outer, 0)

        with scope("owait"):
            for m_ in range(NM):
                for a in range(NS):
                    for i in range(len(OS)):
                        ocp(m_, a, i).wait()

    def fn(x, w_gate, w_up, w_down):
        B, S, _ = x.shape
        xt = x.reshape(M, D).T
        wdt = w_down.T
        out = pl.pallas_call(
            kernel,
            in_specs=[pl.BlockSpec(memory_space=pl.ANY)] * 4,
            out_specs=pl.BlockSpec(memory_space=pl.ANY),
            out_shape=jax.ShapeDtypeStruct((D, M), x.dtype),
            scratch_shapes=[pltpu.VMEM((D, M), bf), pltpu.VMEM((NM, 5, MH // 2, 128), u32),
                            pltpu.VMEM((D, FA), bf), pltpu.VMEM((D, FA), bf), pltpu.VMEM((D, FA), bf),
                            pltpu.VMEM((NF, D, FB), bf), pltpu.VMEM((NF, D, FB), bf), pltpu.VMEM((NF, D, FB), bf),
                            pltpu.VMEM((NM, NS, D, 128), f32),
                            pltpu.VMEM((NF, NQ, KT, 1, 8, 128), f32),
                            pltpu.VMEM((NM, NBLK, KT, 4, 8, 128), f32),
                            pltpu.VMEM((2, MH, 128), f32),
                            pltpu.VMEM((NQ, 2, rt, 128), f32),
                            pltpu.VMEM((MH, 128), f32), pltpu.VMEM((MH, 128), f32),
                            pltpu.VMEM((NTB, MH, 128), bf),
                            pltpu.VMEM((NT * NTA, TA, 128), bf),
                            pltpu.VMEM((4, D // 2, 128), u32),
                            pltpu.VMEM((NM, NS, D, 128), bf),
                            pltpu.SemaphoreType.DMA((7,)), pltpu.SemaphoreType.DMA((1,))],
            compiler_params=pltpu.CompilerParams(
                vmem_limit_bytes=vmem * 1024 * 1024,
                disable_semaphore_checks=bool(nosc),
            ),
        )(xt, w_gate, w_up, wdt)
        return out.T.reshape(B, S, D)
    return fn


_impl = build()


@jax.jit
def pallas_standalone__geglu_ffn__prompt_kernel(
    x: jax.Array,
    w_gate: jax.Array,
    w_up: jax.Array,
    w_down: jax.Array,
):
    return _impl(x, w_gate, w_up, w_down)
```

```python
import jax
import jax.numpy as jnp
from jax import lax
import jax.experimental.pallas as pl
import jax.experimental.pallas.tpu as pltpu

C0 = 0.7978845608028654
C1 = C0 * 0.044715

D, F, M = 576, 4608, 2048
KM, KT, KH = 512, 64, 32
TA = 512
FA, NF, MH = 384, 3, 1024
R = 32
RT = 320
NM, NT, NS = M // MH, M // TA, MH // 128
FB = (F - FA) // NF
NTA, NTB = FA // 128, FB // 128
NQ = NTB * 2
NC = NF * NTB
NBLK = RT // R
HBQ = 2 * NBLK
NHB = NQ * HBQ
NIT = NM * NF
NE = 4
LEAD = 5
HB1, HB2, HB3 = 27, 41, 6
WT, WG, WU, WD = 58, 52, 36, 50
VT = 0.2
FN = (0, 1, 2, NTB - 1)
OS = ((0, 384), (384, D - 384))

f32, bf16, u32, i32 = jnp.float32, jnp.bfloat16, jnp.uint32, jnp.int32


def _geglu2(g, u):
    z = g * (C0 + C1 * (g * g))
    p = g * u
    return p + p * jnp.tanh(z)


def _mm(a, b):
    return jnp.dot(a, b, preferred_element_type=f32)


def _mm_nt(a, b):
    return lax.dot_general(a, b, (((1,), (1,)), ((), ())), preferred_element_type=f32)


def _tile(n, w=128):
    return pl.ds(pl.multiple_of(n * w, w), w)


def _uloop(lo, hi, fn):
    lax.fori_loop(lo, hi, lambda i, c: (fn(i), c)[1], 0, unroll=True)


def _kernel(xt_hbm, wg_hbm, wu_hbm, wdt_hbm, o_hbm,
            xt_s, xs, wga, wua, wda, wgb, wub, wdb, acc_s, wb_s, xb_s, tm_s, tv_s, g_s, j_s, h_s, ha_s,
            wdp, o_s, sem, osem):

    def cp(src, dst, lo, n, s):
        return pltpu.make_async_copy(src.at[:, pl.ds(lo, n)], dst.at[:, pl.ds(lo, n)], sem.at[s])

    def cpr(src, dst, f, r0, nr, s, c0=0, nc=FB):
        return pltpu.make_async_copy(src.at[pl.ds(r0, nr), pl.ds(FA + f * FB + c0, nc)],
                                     dst.at[f, pl.ds(r0, nr), pl.ds(c0, nc)], sem.at[s])

    def wblock(f, s):
        return [cpr(wg_hbm, wgb, f, 0, KM, s), cpr(wu_hbm, wub, f, 0, KM, s), cpr(wdt_hbm, wdb, f, 0, D, s)]

    def gua(c, s):
        return [cp(wg_hbm, wga, c * 128, 128, s), cp(wu_hbm, wua, c * 128, 128, s)]

    gw = ((wg_hbm, wgb), (wu_hbm, wub))
    groups = [
        [cp(xt_hbm, xt_s, 0, 256, 0)],
        gua(0, 1),
        gua(1, 2) + [cp(xt_hbm, xt_s, 256, 256, 2)],
        gua(2, 3) + [cp(xt_hbm, xt_s, TA, TA, 3)] + [cpr(s_, d_, 0, KM, KT, 3, 0, NE * 128) for s_, d_ in gw],
        [cp(wdt_hbm, wda, 0, FA, 4), cp(xt_hbm, xt_s, 2 * TA, 2 * TA, 4)]
        + [cpr(s_, d_, 0, KM, KT, 4, NE * 128, FB - NE * 128) for s_, d_ in gw]
        + [cpr(s_, d_, f, KM, KT, 4) for f in range(1, NF) for s_, d_ in gw],
        wblock(0, 5),
        [c for f in range(1, NF) for c in wblock(f, 6)],
    ]

    def wait(g):
        for c in groups[g]:
            c.wait()

    for g in groups:
        for c in g:
            c.start()

    def xpose(lo, n):
        x = xt_s[:, lo:lo + n].T
        m, r0 = lo // MH, (lo % MH) // 2
        for kt in range(4):
            xs[m, kt, r0:r0 + n // 2, :] = pltpu.bitcast(x[:, kt * 128:(kt + 1) * 128], u32)
        xs[m, 4, r0:r0 + n // 2, :] = jnp.concatenate(
            [pltpu.bitcast(x[:, KM:D], u32), jnp.zeros((n // 2, 128 - KT), u32)], axis=1)
        return x

    class Ties:
        def __init__(self, it, hb0, nhb, cur, nxt, total_w, front, lumps=(), total_v=None):
            self.it, self.masks = it, {}
            self.hb0, self.cur, self.nxt = hb0, cur, nxt
            self.total = nhb * KH
            self.W = total_w * front
            self.w = self.v = 0.0
            self.done = self.k = 0
            self.acc = self.job = None
            self.lumps = [((total_v or total_w) * (0.02 + 0.91 * i / len(lumps)), l) for i, l in enumerate(lumps)]

        def mask(self, rows=R):
            if rows not in self.masks:
                self.masks[rows] = lax.broadcasted_iota(i32, (rows, 128), 1) < (self.it - 1000)
            return self.masks[rows]

        def decode(self, i):
            b = self.hb0 + i
            m, f = self.cur
            if self.nxt is not None:
                wrap = b >= NHB
                b = lax.rem(b, NHB)
                m, f = lax.select(wrap, self.nxt[0], m), lax.select(wrap, self.nxt[1], f)
            q, e = lax.div(b, HBQ), lax.rem(b, HBQ)
            return q, lax.rem(e, 2), lax.div(e, 2), m, f

        def skip(self, w, v=None):
            self.w += w
            self.v += w if v is None else v

        def __call__(self, piece, slot, w, v=None):
            self.skip(w, v)
            if self.lumps and self.v >= self.lumps[0][0]:
                self.lumps.pop(0)[1](lambda x: lax.select(
                    self.mask(x.shape[0]), pltpu.bitcast(piece()[0:x.shape[0]], u32), x))
            target = min(self.total, int(self.total * self.w / self.W))
            while target > self.done:
                if self.job is None:
                    self.job = self.decode(self.done // KH)
                q, half, blk, m, f = self.job
                kk = min(target - self.done, KH - self.k)
                if KH - self.k - kk <= 2:
                    kk = KH - self.k
                ks = pl.ds(half * KH + self.k, kk)
                p = xb_s[m, blk, ks] * wb_s[f, q, ks]
                h2 = (kk + 1) // 2
                acc = jnp.sum(p[0:h2], axis=0)
                if self.acc is not None:
                    acc = acc + self.acc
                if kk > h2:
                    acc = acc + jnp.sum(p[h2:kk], axis=0)
                self.done += kk
                self.k += kk
                self.acc = acc
                a2 = acc.reshape(R, 128)
                if self.k < KH:
                    slot[...] = a2
                    return
                tv_s[q, half, _tile(blk, R), :] = lax.select(self.mask(), piece(), a2)
                self.k, self.acc, self.job = 0, None, None
                if target - self.done <= 2:
                    break

        def store(self, dst, val, w_per_beat):
            for a in range(0, val.shape[0], R):
                self(lambda: val[a:a + R], dst.at[pl.ds(a, R), :], w_per_beat * 2, 2.0)
            dst[...] = val

        def finish(self):
            assert self.done == self.total and not self.lumps

    w_gu = lambda tm, rv: WT * ((tm - rv) / 32) + (WG + WU) * (tm // 16)
    v_gu = lambda tm, rv: VT * ((tm - rv) / 32) + 2 * (tm // 16)

    def gu_unit(tie, xr, tm, rv, q, wg, wu, h_dst, mid=None):
        H = (tm - rv) // 2
        parts = [(0, rv), (0, rv + H), (1, rv), (1, rv + H)]
        res = [_mm(pltpu.bitcast(xr(4, a0, H)[:, 0:KT], bf16), (wg, wu)[w_](KM, D)) for w_, a0 in parts]
        for a in range(0, H, R):
            for pi, ((w_, a0), rs_) in enumerate(zip(parts, res)):
                if pi % 2:
                    tie(lambda: rs_[a:a + R], tm_s.at[w_, pl.ds(a0 + a, R), :], WT / 2, VT / 2)
                else:
                    tie.skip(WT / 2, VT / 2)
        for (w_, a0), rs_ in zip(parts, res):
            tm_s[w_, a0:a0 + H, :] = rs_

        def full(w_):
            xmain = jnp.concatenate([pltpu.bitcast(xr(kt, 0, tm), bf16) for kt in range(4)], axis=1)
            main = _mm(xmain, (wg, wu)[w_](0, KM))
            if not rv:
                return main + tm_s[w_, 0:tm]
            return jnp.concatenate([(main[0:rv] + tv_s[q + w_, 0]) + tv_s[q + w_, 1],
                                    main[rv:tm] + tm_s[w_, rv:tm]], axis=0)
        tie.store(g_s.at[0:tm], full(0), WG)
        if mid is not None:
            mid()
        u = full(1)
        tie.store(j_s.at[0:tm], u, WU)
        h_dst[...] = _geglu2(g_s[0:tm], u).astype(bf16)
        tie.finish()

    def dn_unit(tie, wd, h, m):
        for t in range(MH // 512):
            p_ = _mm_nt(wd(), h(t))
            for a in range(3):
                acc_s[m, 4 * t + a] += p_[:, a * 128:(a + 1) * 128]
            dst = acc_s.at[m, 4 * t + 3]
            tie.store(dst, dst[...] + p_[:, 384:512], WD)

    def d3_unit(tie, tt):
        cat = lambda xs_: jnp.concatenate(xs_, axis=1) if len(xs_) > 1 else xs_[0]
        m, a0 = lax.div(tt, 2), lax.rem(tt, 2) * 4
        seen = set()
        for rnd in (((0, (0, 1, 2)), (1, (0,))), ((1, (1, 2)), (2, (0, 1))), ((2, (2,)), (3, (0, 1, 2)))):
            vs = []
            for a, ks in rnd:
                v = _mm_nt(wda[:, ks[0] * 128:(ks[-1] + 1) * 128],
                           cat([ha_s[tt * NTA + n, a * 128:(a + 1) * 128, :] for n in ks]))
                dst = acc_s.at[m, a0 + a]
                vs.append((dst, dst[...] + v if a in seen else v))
            for r0 in range(0, D, R):
                for dst, v in vs:
                    tie(lambda: v[r0:r0 + R], dst.at[pl.ds(r0, R), :], 1.0)
            for dst, v in vs:
                dst[...] = v
            seen.update(a for a, _ in rnd)
        tie.finish()

    def xb_lump(m, blk, k0, nk):
        def emit(pin):
            src = pin(xs[m, 4, _tile(blk, 16), :])
            b = jnp.stack([jnp.broadcast_to(src[:, k:k + 1], (16, 128)) for k in range(k0, k0 + nk)])
            xb_s[m, blk, k0:k0 + nk] = pltpu.bitcast(b, bf16).astype(f32).reshape(nk, 4, 8, 128)
        return emit

    def wb_lump(c, which, k0, nk):
        def emit(pin):
            f, n = lax.div(c, NTB), lax.rem(c, NTB)
            src = pin(pltpu.bitcast((wgb, wub)[which][f, KM + k0:KM + k0 + nk, _tile(n)], u32))
            v = pltpu.bitcast(src, bf16).astype(f32)
            wb_s[f, 2 * n + which, k0:k0 + nk, 0] = jnp.stack(
                [jnp.broadcast_to(v[k:k + 1], (8, 128)) for k in range(nk)])
        return emit

    def wb_lumps(c, which):
        return [wb_lump(c, which, k0, 16) for k0 in range(0, KT, 16)]

    def phase_a(it):
        zero = jnp.zeros((), i32)

        def gu_v(x, lo, n, rr, r0):
            wg, wu = wga[:, lo:lo + n], wua[:, lo:lo + n]
            for a in range(0, x.shape[0], rr):
                h = _geglu2(_mm(x[a:a + rr], wg), _mm(x[a:a + rr], wu)).astype(bf16)
                for c in range(n // 128):
                    ha_s[lo // 128 + c, r0 + a:r0 + a + rr, :] = h[:, c * 128:(c + 1) * 128]

        def mix(a, b):
            out = [(i / len(a), x) for i, x in enumerate(a)] + [((i + .5) / len(b), x) for i, x in enumerate(b)]
            return [x for _, x in sorted(out, key=lambda e: e[0])]

        def xl_at(m, blk0, nb):
            return [xb_lump(m, jnp.minimum(blk0 + i, NBLK - 1), k0, 8) for i in range(nb) for k0 in range(0, KT, 8)]

        def wl_at(i0, n):
            return [l for i in range(n) for l in wb_lumps(jnp.minimum(NE + i0 + i // 2, NC - 1), i % 2)]

        def gu_a(u, m, lumps, hb0=0, nhb=0):
            cs, tt = _tile(lax.rem(u, NTA)), lax.div(u, NTA)
            tie = Ties(it, hb0, nhb, (zero, zero), None, w_gu(TA, 0), 0.98, lumps, v_gu(TA, 0))
            row0 = lax.rem(tt, 2) * (TA // 2)
            xr = lambda kt, a, n: xs[m, kt, pl.ds(pl.multiple_of(row0 + a // 2, 8), n // 2), :]
            gu_unit(tie, xr, TA, 0, 0, lambda a, b: wga[a:b, cs], lambda a, b: wua[a:b, cs], ha_s.at[u])

        def d3_a(tt, lumps, hb0, nhb):
            d3_unit(Ties(it, hb0, nhb, (zero, zero), None, 6 * (D // R), 0.98, lumps), tt)

        nopin = lambda v: v
        wait(0)
        xa = xpose(0, 256)
        xb_lump(0, 0, 0, KT)(nopin)
        wait(1)
        gu_v(xa, 0, 128, 128, 0)
        xb_lump(0, 1, 0, KT)(nopin)
        wait(2)
        xb = xpose(256, 256)
        gu_v(xa, 128, 128, 128, 0)
        gu_v(xb, 0, 256, 256, 256)
        wait(3)
        xpose(TA, TA)
        _uloop(2, 6, lambda u: gu_a(u, 0, mix(xl_at(0, 2 * u - 2, 2), wb_lumps(u - 2, 0) + wb_lumps(u - 2, 1))))
        wait(4)
        w1, w2, w3 = 8, 6, 4
        m1, m2, m3 = 13, 8, 13
        assert 2 * w1 + 6 * w2 + 2 * w3 >= 2 * (NC - NE) and 6 + 2 * 2 >= NBLK
        assert 2 * m1 + 6 * m2 + 2 * m3 >= LEAD * HBQ
        xpose(2 * TA, TA)
        xpose(3 * TA, TA)
        _uloop(0, 2, lambda tt: d3_a(tt, wl_at(tt * (w1 // 2), w1), tt * m1, m1))
        _uloop(6, 12, lambda u: gu_a(u, 1, mix(xl_at(1, u - 6, 1), wl_at(w1 + (u - 6) * (w2 // 2), w2)),
                                     2 * m1 + (u - 6) * m2, m2))
        _uloop(2, 4, lambda tt: d3_a(
            tt, mix(xl_at(1, 6 + (tt - 2) * 2, 2), wl_at(w1 + 3 * w2 + (tt - 2) * (w3 // 2), w3)),
            jnp.minimum(2 * m1 + 6 * m2 + (tt - 2) * m3, LEAD * HBQ - m3), m3))
        wait(5)

    def ocp(m_, a, i):
        rows = pl.ds(*OS[i])
        return pltpu.make_async_copy(o_s.at[m_, a, rows], o_hbm.at[rows, _tile(m_ * NS + a)], osem.at[0])

    assert 4 * HB1 + (NTB - 4) * HB2 + NS * HB3 >= NHB
    for n in range(NTB):
        assert LEAD * HBQ + min(n, 4) * HB1 + max(n - 4, 0) * HB2 >= (2 * n + 2) * HBQ

    def body(j):
        cur = (lax.bitwise_and(j, 1), lax.shift_right_logical(j, 1))
        jn = jnp.minimum(j + 1, NIT - 1)
        nxt = (lax.bitwise_and(jn, 1), lax.shift_right_logical(jn, 1))
        m, f = cur

        @pl.when(j == 1)
        def _():
            wait(6)

        base = LEAD * HBQ
        hu = h_s.bitcast(u32)
        hld = lambda n, i, sz: pltpu.bitcast(hu[n, _tile(i, sz // 2), :], bf16)
        xr = lambda kt, a, n_: xs[m, kt, a // 2:(a + n_) // 2, :]

        def unit(n, with_d):
            cs = _tile(n)
            hb0 = base + (4 * HB1 + (n - 4) * HB2 if with_d else n * HB1)
            tie = Ties(j, hb0, HB2 if with_d else HB1, cur, nxt if with_d else None,
                       w_gu(MH, RT) + (2 * (D // 16) * WD if with_d else 0), 0.997)
            mid = None
            if with_d:
                mid = lambda: dn_unit(tie, lambda: wdb[f, :, _tile(n - 1)], lambda t: hld(n - 1, t, 512), m)
            gu_unit(tie, xr, MH, RT, 2 * n, lambda a, b: wgb[f, a:b, cs], lambda a, b: wub[f, a:b, cs],
                    h_s.at[n], mid)

        def final(a):
            hb0 = jnp.minimum(base + 4 * HB1 + (NTB - 4) * HB2 + a * HB3, base + NHB - HB3)
            tie = Ties(j, hb0, HB3, cur, nxt, D // 16, 0.98)
            wd = jnp.concatenate([pltpu.bitcast(wdp[i], bf16) for i in range(4)], axis=1)
            h = jnp.concatenate([hld(n, a, 128) for n in FN], axis=1)
            dst = acc_s.at[m, a]
            acc = dst[...] + _mm_nt(wd, h)
            tie.store(dst, acc, 1.0)
            tie.finish()
            for i, (r0, nr) in enumerate(OS):
                o_s[m, a, r0:r0 + nr] = (0.5 * acc[r0:r0 + nr]).astype(bf16)
                for m_ in range(NM):
                    @pl.when(j == NIT - NM + m_)
                    def _():
                        ocp(m_, a, i).start()

        _uloop(0, 4, lambda n: unit(n, False))
        _uloop(4, NTB, lambda n: unit(n, True))
        for i, n in enumerate(FN):
            wdp[i] = pltpu.bitcast(wdb[f, :, n * 128:(n + 1) * 128], u32)
        _uloop(0, NS, final)

    def outer(it, carry):
        lax.cond(it == 0, lambda: phase_a(it), lambda: body(it - 1))
        return carry
    lax.fori_loop(0, NIT + 1, outer, 0)

    for m_ in range(NM):
        for a in range(NS):
            for i in range(len(OS)):
                ocp(m_, a, i).wait()


@jax.jit
def pallas_standalone__geglu_ffn__prompt_kernel(
    x: jax.Array,
    w_gate: jax.Array,
    w_up: jax.Array,
    w_down: jax.Array,
):
    B, S, _ = x.shape
    assert (B * S, x.shape[2], w_gate.shape[1]) == (M, D, F)
    out_t = pl.pallas_call(
        _kernel,
        in_specs=[pl.BlockSpec(memory_space=pl.ANY)] * 4,
        out_specs=pl.BlockSpec(memory_space=pl.ANY),
        out_shape=jax.ShapeDtypeStruct((D, M), x.dtype),
        scratch_shapes=[
            pltpu.VMEM((D, M), bf16),
            pltpu.VMEM((NM, 5, MH // 2, 128), u32),
            pltpu.VMEM((D, FA), bf16), pltpu.VMEM((D, FA), bf16), pltpu.VMEM((D, FA), bf16),
            pltpu.VMEM((NF, D, FB), bf16), pltpu.VMEM((NF, D, FB), bf16), pltpu.VMEM((NF, D, FB), bf16),
            pltpu.VMEM((NM, NS, D, 128), f32),
            pltpu.VMEM((NF, NQ, KT, 1, 8, 128), f32),
            pltpu.VMEM((NM, NBLK, KT, 4, 8, 128), f32),
            pltpu.VMEM((2, MH, 128), f32),
            pltpu.VMEM((NQ, 2, RT, 128), f32),
            pltpu.VMEM((MH, 128), f32), pltpu.VMEM((MH, 128), f32),
            pltpu.VMEM((NTB, MH, 128), bf16),
            pltpu.VMEM((NT * NTA, TA, 128), bf16),
            pltpu.VMEM((4, D // 2, 128), u32),
            pltpu.VMEM((NM, NS, D, 128), bf16),
            pltpu.SemaphoreType.DMA((7,)), pltpu.SemaphoreType.DMA((1,))],
        compiler_params=pltpu.CompilerParams(
            vmem_limit_bytes=120 * 1024 * 1024,
            disable_semaphore_checks=True,
        ),
    )(x.reshape(M, D).T, w_gate, w_up, w_down.T)
    return out_t.T.reshape(B, S, D)
```

```python
import jax
import jax.numpy as jnp
from jax import lax
import jax.experimental.pallas as pl
import jax.experimental.pallas.tpu as pltpu

C0 = 0.7978845608028654
C1 = C0 * 0.044715

D, F, M = 576, 4608, 2048
KM, KT, KH = 512, 64, 32
TA = 512
FA, NF, MH = 384, 3, 1024
R = 32
RT = 320
NM, NT, NS = M // MH, M // TA, MH // 128
FB = (F - FA) // NF
NTA, NTB = FA // 128, FB // 128
NQ = NTB * 2
NC = NF * NTB
NBLK = RT // R
HBQ = 2 * NBLK
NHB = NQ * HBQ
NIT = NM * NF
NE = 4
LEAD = 5
HB1, HB2, HB3 = 27, 41, 6
WT, WG, WU, WD = 58, 52, 36, 50
WTA = 20
VT = 0.2
FN = (0, 1, 2, NTB - 1)
OS = ((0, 384), (384, D - 384))

f32, bf16, u32, i32 = jnp.float32, jnp.bfloat16, jnp.uint32, jnp.int32


def _geglu2(g, u):
    z = g * (C0 + C1 * (g * g))
    p = g * u
    return p + p * jnp.tanh(z)


def _mm(a, b):
    return jnp.dot(a, b, preferred_element_type=f32)


def _mm_nt(a, b):
    return lax.dot_general(a, b, (((1,), (1,)), ((), ())), preferred_element_type=f32)


def _tile(n, w=128):
    return pl.ds(pl.multiple_of(n * w, w), w)


def _uloop(lo, hi, fn):
    lax.fori_loop(lo, hi, lambda i, c: (fn(i), c)[1], 0, unroll=True)


def _kernel(xt_hbm, wg_hbm, wu_hbm, wdt_hbm, o_hbm,
            xt_s, xs, wga, wua, wda, wgb, wub, wdb, acc_s, wb_s, xb_s, tm_s, tv_s, g_s, j_s, h_s, ha_s,
            wdp, o_s, sem, osem):

    def cp(src, dst, lo, n, s):
        return pltpu.make_async_copy(src.at[:, pl.ds(lo, n)], dst.at[:, pl.ds(lo, n)], sem.at[s])

    def cpr(src, dst, f, r0, nr, s, c0=0, nc=FB):
        return pltpu.make_async_copy(src.at[pl.ds(r0, nr), pl.ds(FA + f * FB + c0, nc)],
                                     dst.at[f, pl.ds(r0, nr), pl.ds(c0, nc)], sem.at[s])

    def wblock(f, s):
        return [cpr(wg_hbm, wgb, f, 0, KM, s), cpr(wu_hbm, wub, f, 0, KM, s), cpr(wdt_hbm, wdb, f, 0, D, s)]

    gw = ((wg_hbm, wgb), (wu_hbm, wub))
    groups = [
        [cp(xt_hbm, xt_s, 0, 256, 0)],
        [cp(wg_hbm, wga, 0, 256, 1)],
        [cp(wu_hbm, wua, 0, 256, 2), cp(xt_hbm, xt_s, 256, 256, 2)],
        [cp(wg_hbm, wga, 256, 128, 3), cp(wu_hbm, wua, 256, 128, 3), cp(xt_hbm, xt_s, TA, TA, 3)]
        + [cpr(s_, d_, 0, KM, KT, 3, 0, NE * 128) for s_, d_ in gw],
        [cp(wdt_hbm, wda, 0, FA, 4), cp(xt_hbm, xt_s, 2 * TA, 2 * TA, 4)]
        + [cpr(s_, d_, 0, KM, KT, 4, NE * 128, FB - NE * 128) for s_, d_ in gw]
        + [cpr(s_, d_, f, KM, KT, 4) for f in range(1, NF) for s_, d_ in gw],
        wblock(0, 5),
        [c for f in range(1, NF) for c in wblock(f, 6)],
    ]

    def wait(g):
        for c in groups[g]:
            c.wait()

    for g in groups:
        for c in g:
            c.start()

    def xpose(lo, n):
        x = xt_s[:, lo:lo + n].T
        m, r0 = lo // MH, (lo % MH) // 2
        for kt in range(4):
            xs[m, kt, r0:r0 + n // 2, :] = pltpu.bitcast(x[:, kt * 128:(kt + 1) * 128], u32)
        xs[m, 4, r0:r0 + n // 2, :] = jnp.concatenate(
            [pltpu.bitcast(x[:, KM:D], u32), jnp.zeros((n // 2, 128 - KT), u32)], axis=1)
        return x

    class Ties:
        def __init__(self, it, hb0, nhb, cur, nxt, total_w, front, lumps=(), total_v=None):
            self.it, self.masks = it, {}
            self.hb0, self.cur, self.nxt = hb0, cur, nxt
            self.total = nhb * KH
            self.W = total_w * front
            self.w = self.v = 0.0
            self.done = self.k = 0
            self.acc = self.job = None
            self.lumps = [((total_v or total_w) * (0.02 + 0.91 * i / len(lumps)), l) for i, l in enumerate(lumps)]

        def mask(self, rows=R):
            if rows not in self.masks:
                self.masks[rows] = lax.broadcasted_iota(i32, (rows, 128), 1) < (self.it - 1000)
            return self.masks[rows]

        def decode(self, i):
            b = self.hb0 + i
            m, f = self.cur
            if self.nxt is not None:
                wrap = b >= NHB
                b = lax.rem(b, NHB)
                m, f = lax.select(wrap, self.nxt[0], m), lax.select(wrap, self.nxt[1], f)
            q, e = lax.div(b, HBQ), lax.rem(b, HBQ)
            return q, lax.rem(e, 2), lax.div(e, 2), m, f

        def skip(self, w, v=None):
            self.w += w
            self.v += w if v is None else v

        def __call__(self, piece, slot, w, v=None):
            self.skip(w, v)
            if self.lumps and self.v >= self.lumps[0][0]:
                self.lumps.pop(0)[1](lambda x: lax.select(
                    self.mask(x.shape[0]), pltpu.bitcast(piece()[0:x.shape[0]], u32), x))
            target = min(self.total, int(self.total * self.w / self.W))
            while target > self.done:
                if self.job is None:
                    self.job = self.decode(self.done // KH)
                q, half, blk, m, f = self.job
                kk = min(target - self.done, KH - self.k)
                if KH - self.k - kk <= 2:
                    kk = KH - self.k
                ks = pl.ds(half * KH + self.k, kk)
                p = xb_s[m, blk, ks] * wb_s[f, q, ks]
                h2 = (kk + 1) // 2
                acc = jnp.sum(p[0:h2], axis=0)
                if self.acc is not None:
                    acc = acc + self.acc
                if kk > h2:
                    acc = acc + jnp.sum(p[h2:kk], axis=0)
                self.done += kk
                self.k += kk
                self.acc = acc
                a2 = acc.reshape(R, 128)
                if self.k < KH:
                    slot[...] = a2
                    return
                tv_s[q, half, _tile(blk, R), :] = lax.select(self.mask(), piece(), a2)
                self.k, self.acc, self.job = 0, None, None
                if target - self.done <= 2:
                    break

        def store(self, dst, val, w_per_beat):
            for a in range(0, val.shape[0], R):
                self(lambda: val[a:a + R], dst.at[pl.ds(a, R), :], w_per_beat * 2, 2.0)
            dst[...] = val

        def finish(self):
            assert self.done == self.total and not self.lumps

    w_gu = lambda tm, rv, wt=WT: wt * ((tm - rv) / 32) + (WG + WU) * (tm // 16)
    v_gu = lambda tm, rv: VT * ((tm - rv) / 32) + 2 * (tm // 16)

    def gu_unit(tie, xr, tm, rv, q, wg, wu, h_dst, mid=None, wt=WT):
        H = (tm - rv) // 2
        parts = [(0, rv), (0, rv + H), (1, rv), (1, rv + H)]
        res = [_mm(pltpu.bitcast(xr(4, a0, H)[:, 0:KT], bf16), (wg, wu)[w_](KM, D)) for w_, a0 in parts]
        for a in range(0, H, R):
            for pi, ((w_, a0), rs_) in enumerate(zip(parts, res)):
                if pi % 2:
                    tie(lambda: rs_[a:a + R], tm_s.at[w_, pl.ds(a0 + a, R), :], wt / 2, VT / 2)
                else:
                    tie.skip(wt / 2, VT / 2)
        for (w_, a0), rs_ in zip(parts, res):
            tm_s[w_, a0:a0 + H, :] = rs_

        def full(w_):
            xmain = jnp.concatenate([pltpu.bitcast(xr(kt, 0, tm), bf16) for kt in range(4)], axis=1)
            main = _mm(xmain, (wg, wu)[w_](0, KM))
            if not rv:
                return main + tm_s[w_, 0:tm]
            return jnp.concatenate([(main[0:rv] + tv_s[q + w_, 0]) + tv_s[q + w_, 1],
                                    main[rv:tm] + tm_s[w_, rv:tm]], axis=0)
        tie.store(g_s.at[0:tm], full(0), WG)
        if mid is not None:
            mid()
        u = full(1)
        tie.store(j_s.at[0:tm], u, WU)
        h_dst[...] = _geglu2(g_s[0:tm], u).astype(bf16)
        tie.finish()

    def dn_unit(tie, wd, h, m):
        for t in range(MH // 512):
            p_ = _mm_nt(wd(), h(t))
            for a in range(3):
                acc_s[m, 4 * t + a] += p_[:, a * 128:(a + 1) * 128]
            dst = acc_s.at[m, 4 * t + 3]
            tie.store(dst, dst[...] + p_[:, 384:512], WD)

    def d3_unit(tie, tt):
        cat = lambda xs_: jnp.concatenate(xs_, axis=1) if len(xs_) > 1 else xs_[0]
        m, a0 = lax.div(tt, 2), lax.rem(tt, 2) * 4
        hau = ha_s.bitcast(u32)
        seen = set()
        for rnd in (((0, (0, 1, 2)), (1, (0,))), ((1, (1, 2)), (2, (0, 1))), ((2, (2,)), (3, (0, 1, 2)))):
            vs = []
            for a, ks in rnd:
                v = _mm_nt(cat([pltpu.bitcast(wdp[n], bf16) for n in ks]),
                           cat([pltpu.bitcast(hau[tt * NTA + n, a * 64:(a + 1) * 64, :], bf16) for n in ks]))
                dst = acc_s.at[m, a0 + a]
                vs.append((dst, dst[...] + v if a in seen else v))
            for r0 in range(0, D, R):
                for dst, v in vs:
                    tie(lambda: v[r0:r0 + R], dst.at[pl.ds(r0, R), :], 1.0)
            for dst, v in vs:
                dst[...] = v
            seen.update(a for a, _ in rnd)
        tie.finish()

    def xb_lump(m, blk, k0, nk):
        def emit(pin):
            src = pin(xs[m, 4, _tile(blk, 16), :])
            b = jnp.stack([jnp.broadcast_to(src[:, k:k + 1], (16, 128)) for k in range(k0, k0 + nk)])
            xb_s[m, blk, k0:k0 + nk] = pltpu.bitcast(b, bf16).astype(f32).reshape(nk, 4, 8, 128)
        return emit

    def wb_lump(c, which, k0, nk):
        def emit(pin):
            f, n = lax.div(c, NTB), lax.rem(c, NTB)
            src = pin(pltpu.bitcast((wgb, wub)[which][f, KM + k0:KM + k0 + nk, _tile(n)], u32))
            v = pltpu.bitcast(src, bf16).astype(f32)
            wb_s[f, 2 * n + which, k0:k0 + nk, 0] = jnp.stack(
                [jnp.broadcast_to(v[k:k + 1], (8, 128)) for k in range(nk)])
        return emit

    def wb_lumps(c, which):
        return [wb_lump(c, which, k0, 16) for k0 in range(0, KT, 16)]

    def phase_a(it):
        zero = jnp.zeros((), i32)

        def put_h(g, u, r0):
            h = _geglu2(g, u).astype(bf16)
            for c in range(2):
                ha_s[c, r0:r0 + h.shape[0], :] = h[:, c * 128:(c + 1) * 128]

        def mix(a, b):
            out = [(i / len(a), x) for i, x in enumerate(a)] + [((i + .5) / len(b), x) for i, x in enumerate(b)]
            return [x for _, x in sorted(out, key=lambda e: e[0])]

        def xl_at(m, blk0, nb):
            return [xb_lump(m, jnp.minimum(blk0 + i, NBLK - 1), k0, 8) for i in range(nb) for k0 in range(0, KT, 8)]

        def wl_at(i0, n):
            return [l for i in range(n) for l in wb_lumps(jnp.minimum(NE + i0 + i // 2, NC - 1), i % 2)]

        def gu_a(u, m, lumps, hb0=0, nhb=0):
            cs, tt = _tile(lax.rem(u, NTA)), lax.div(u, NTA)
            tie = Ties(it, hb0, nhb, (zero, zero), None, w_gu(TA, 0, WTA), 0.98, lumps, v_gu(TA, 0))
            row0 = lax.rem(tt, 2) * (TA // 2)
            xr = lambda kt, a, n: xs[m, kt, pl.ds(pl.multiple_of(row0 + a // 2, 8), n // 2), :]
            gu_unit(tie, xr, TA, 0, 0, lambda a, b: wga[a:b, cs], lambda a, b: wua[a:b, cs], ha_s.at[u], None, WTA)

        def d3_a(tt, lumps, hb0, nhb):
            d3_unit(Ties(it, hb0, nhb, (zero, zero), None, 6 * (D // R), 0.98, lumps), tt)

        nopin = lambda v: v
        wait(0)
        xa = xpose(0, 256)
        xb_lump(0, 0, 0, KT)(nopin)
        wait(1)
        ga = [_mm(xa[a:a + 128], wga[:, 0:256]) for a in (0, 128)]
        xb_lump(0, 1, 0, KT)(nopin)
        wait(2)
        xb = xpose(256, 256)
        for i, a in enumerate((0, 128)):
            put_h(ga[i], _mm(xa[a:a + 128], wua[:, 0:256]), a)
        wg2, wu2 = wga[:, 0:256], wua[:, 0:256]
        put_h(_mm(xb, wg2), _mm(xb, wu2), 256)
        wait(3)
        xpose(TA, TA)
        _uloop(2, 6, lambda u: gu_a(u, 0, mix(xl_at(0, 2 * u - 2, 2), wb_lumps(u - 2, 0) + wb_lumps(u - 2, 1))))
        wait(4)
        w1, w2, w3 = 8, 6, 4
        m1, m2, m3 = 13, 8, 13
        assert 2 * w1 + 6 * w2 + 2 * w3 >= 2 * (NC - NE) and 6 + 2 * 2 >= NBLK
        assert 2 * m1 + 6 * m2 + 2 * m3 >= LEAD * HBQ
        for n in range(NTA):
            wdp[n] = pltpu.bitcast(wda[:, n * 128:(n + 1) * 128], u32)
        xpose(2 * TA, TA)
        xpose(3 * TA, TA)
        _uloop(0, 2, lambda tt: d3_a(tt, wl_at(tt * (w1 // 2), w1), tt * m1, m1))
        _uloop(6, 12, lambda u: gu_a(u, 1, mix(xl_at(1, u - 6, 1), wl_at(w1 + (u - 6) * (w2 // 2), w2)),
                                     2 * m1 + (u - 6) * m2, m2))
        _uloop(2, 4, lambda tt: d3_a(
            tt, mix(xl_at(1, 6 + (tt - 2) * 2, 2), wl_at(w1 + 3 * w2 + (tt - 2) * (w3 // 2), w3)),
            jnp.minimum(2 * m1 + 6 * m2 + (tt - 2) * m3, LEAD * HBQ - m3), m3))
        wait(5)

    def ocp(m_, a, i):
        rows = pl.ds(*OS[i])
        return pltpu.make_async_copy(o_s.at[m_, a, rows], o_hbm.at[rows, _tile(m_ * NS + a)], osem.at[0])

    assert 4 * HB1 + (NTB - 4) * HB2 + NS * HB3 >= NHB
    for n in range(NTB):
        assert LEAD * HBQ + min(n, 4) * HB1 + max(n - 4, 0) * HB2 >= (2 * n + 2) * HBQ

    def body(j):
        cur = (lax.bitwise_and(j, 1), lax.shift_right_logical(j, 1))
        jn = jnp.minimum(j + 1, NIT - 1)
        nxt = (lax.bitwise_and(jn, 1), lax.shift_right_logical(jn, 1))
        m, f = cur

        @pl.when(j == 1)
        def _():
            wait(6)

        base = LEAD * HBQ
        hu = h_s.bitcast(u32)
        hld = lambda n, i, sz: pltpu.bitcast(hu[n, _tile(i, sz // 2), :], bf16)
        xr = lambda kt, a, n_: xs[m, kt, a // 2:(a + n_) // 2, :]

        def unit(n, with_d):
            cs = _tile(n)
            hb0 = base + (4 * HB1 + (n - 4) * HB2 if with_d else n * HB1)
            tie = Ties(j, hb0, HB2 if with_d else HB1, cur, nxt if with_d else None,
                       w_gu(MH, RT) + (2 * (D // 16) * WD if with_d else 0), 0.997)
            mid = None
            if with_d:
                mid = lambda: dn_unit(tie, lambda: wdb[f, :, _tile(n - 1)], lambda t: hld(n - 1, t, 512), m)
            gu_unit(tie, xr, MH, RT, 2 * n, lambda a, b: wgb[f, a:b, cs], lambda a, b: wub[f, a:b, cs],
                    h_s.at[n], mid)

        def final(a):
            hb0 = jnp.minimum(base + 4 * HB1 + (NTB - 4) * HB2 + a * HB3, base + NHB - HB3)
            tie = Ties(j, hb0, HB3, cur, nxt, D // 16, 0.98)
            wd = jnp.concatenate([pltpu.bitcast(wdp[i], bf16) for i in range(4)], axis=1)
            h = jnp.concatenate([hld(n, a, 128) for n in FN], axis=1)
            dst = acc_s.at[m, a]
            acc = dst[...] + _mm_nt(wd, h)
            tie.store(dst, acc, 1.0)
            tie.finish()
            for i, (r0, nr) in enumerate(OS):
                o_s[m, a, r0:r0 + nr] = (0.5 * acc[r0:r0 + nr]).astype(bf16)
                for m_ in range(NM):
                    @pl.when(j == NIT - NM + m_)
                    def _():
                        ocp(m_, a, i).start()

        _uloop(0, 4, lambda n: unit(n, False))
        _uloop(4, NTB, lambda n: unit(n, True))
        for i, n in enumerate(FN):
            wdp[i] = pltpu.bitcast(wdb[f, :, n * 128:(n + 1) * 128], u32)
        _uloop(0, NS, final)

    def outer(it, carry):
        lax.cond(it == 0, lambda: phase_a(it), lambda: body(it - 1))
        return carry
    lax.fori_loop(0, NIT + 1, outer, 0)

    for m_ in range(NM):
        for a in range(NS):
            for i in range(len(OS)):
                ocp(m_, a, i).wait()


@jax.jit
def pallas_standalone__geglu_ffn__prompt_kernel(
    x: jax.Array,
    w_gate: jax.Array,
    w_up: jax.Array,
    w_down: jax.Array,
):
    B, S, _ = x.shape
    assert (B * S, x.shape[2], w_gate.shape[1]) == (M, D, F)
    out_t = pl.pallas_call(
        _kernel,
        in_specs=[pl.BlockSpec(memory_space=pl.ANY)] * 4,
        out_specs=pl.BlockSpec(memory_space=pl.ANY),
        out_shape=jax.ShapeDtypeStruct((D, M), x.dtype),
        scratch_shapes=[
            pltpu.VMEM((D, M), bf16),
            pltpu.VMEM((NM, 5, MH // 2, 128), u32),
            pltpu.VMEM((D, FA), bf16), pltpu.VMEM((D, FA), bf16), pltpu.VMEM((D, FA), bf16),
            pltpu.VMEM((NF, D, FB), bf16), pltpu.VMEM((NF, D, FB), bf16), pltpu.VMEM((NF, D, FB), bf16),
            pltpu.VMEM((NM, NS, D, 128), f32),
            pltpu.VMEM((NF, NQ, KT, 1, 8, 128), f32),
            pltpu.VMEM((NM, NBLK, KT, 4, 8, 128), f32),
            pltpu.VMEM((2, MH, 128), f32),
            pltpu.VMEM((NQ, 2, RT, 128), f32),
            pltpu.VMEM((MH, 128), f32), pltpu.VMEM((MH, 128), f32),
            pltpu.VMEM((NTB, MH, 128), bf16),
            pltpu.VMEM((NT * NTA, TA, 128), bf16),
            pltpu.VMEM((4, D // 2, 128), u32),
            pltpu.VMEM((NM, NS, D, 128), bf16),
            pltpu.SemaphoreType.DMA((7,)), pltpu.SemaphoreType.DMA((1,))],
        compiler_params=pltpu.CompilerParams(
            vmem_limit_bytes=100 * 1024 * 1024,
            disable_semaphore_checks=True,
        ),
    )(x.reshape(M, D).T, w_gate, w_up, w_down.T)
    return out_t.T.reshape(B, S, D)
```
